```python
import jax
import jax.numpy as jnp

def _softmax(x, axis=-1):
    return jax.nn.softmax(x, axis=axis)

def _gelu(x):
    return jax.nn.gelu(x, approximate=True)

def _silu(x):
    return jax.nn.silu(x)

def _sigmoid(x):
    return jax.nn.sigmoid(x)

def _layernorm(x, axis=-1, eps=1e-05):
    m = jnp.mean(x, axis=axis, keepdims=True)
    v = jnp.var(x, axis=axis, keepdims=True)
    return (x - m) / jnp.sqrt(v + eps)

def _scatter_add(tgt, idx, src, axis=0):
    return tgt.at[idx].add(src)

def _segment_sum(src, seg, n):
    return jax.ops.segment_sum(src, seg, n)

class _Rng:

    def __init__(self, key):
        self._k = key

    def _next(self):
        self._k, sub = jax.random.split(self._k)
        return sub

    def normal(self, shape):
        return jax.random.normal(self._next(), shape, dtype=jnp.bfloat16)

    def randint(self, lo, hi, shape):
        return jax.random.randint(self._next(), shape, lo, hi, dtype=jnp.int32)

    def uniform(self, shape, lo=0.0, hi=1.0):
        return jax.random.uniform(self._next(), shape, jnp.bfloat16, lo, hi)

    def permutation(self, n):
        return jax.random.permutation(self._next(), n)
kernel_name = 'interleave_layers__memory_aug_recurrent_mem_tr__linear_kernel_hedgehog__prompt'

def setup_inputs():
    _rng = _Rng(jax.random.key(int.from_bytes(__import__("os").urandom(4), "little")))
    _w = lambda a: (lambda t: t.astype(jnp.bfloat16) if jnp.issubdtype(t.dtype, jnp.floating) else t)(jnp.asarray(a))

    def _A_setup():
        B, S, Dm = (1, 2048, 640)
        H, Dh = (32, 192)
        M, seg = (8, 32)
        seg = min(seg, S)
        S = S // seg * seg
        return {'x': _w((lambda *s: _rng.normal(s) * 0.05)(B, S, Dm)), 'mem0': _w((lambda *s: _rng.normal(s) * 0.05)(B, M, Dm)), 'Wq': _w((lambda *s: _rng.normal(s) * 0.05)(Dm, H, Dh) * Dm ** (-0.5)), 'Wk': _w((lambda *s: _rng.normal(s) * 0.05)(Dm, H, Dh) * Dm ** (-0.5)), 'Wv': _w((lambda *s: _rng.normal(s) * 0.05)(Dm, H, Dh) * Dm ** (-0.5)), 'Wo': _w((lambda *s: _rng.normal(s) * 0.05)(H, Dh, Dm) * (H * Dh) ** (-0.5)), 'seg_len': seg}
    _A_in = _A_setup()

    def _B_setup():
        B, S, D, H = (1, 2048, 640, 32)
        Dh = D // H
        return {'x': _w((lambda *s: _rng.normal(s) * 0.05)(B, S, D)), 'wqkv': _w((lambda *s: _rng.normal(s) * 0.05)(D, 3 * D)), 'w_phi': _w((lambda *s: _rng.normal(s) * 0.05)(H, Dh, Dh) * Dh ** (-0.5)), 'wo': _w((lambda *s: _rng.normal(s) * 0.05)(D, D))}
    _B_in = _B_setup()
    return {'A_x': _A_in['x'], 'A_mem0': _A_in['mem0'], 'A_Wq': _A_in['Wq'], 'A_Wk': _A_in['Wk'], 'A_Wv': _A_in['Wv'], 'A_Wo': _A_in['Wo'], 'A_seg_len': _A_in['seg_len'], 'B_x': _B_in['x'], 'B_wqkv': _B_in['wqkv'], 'B_w_phi': _B_in['w_phi'], 'B_wo': _B_in['wo']}

def reference(A_x, A_mem0, A_Wq, A_Wk, A_Wv, A_Wo, A_seg_len, B_x, B_wqkv, B_w_phi, B_wo):

    def _A_ref(x, mem0, Wq, Wk, Wv, Wo, seg_len):
        B, S, Dm = x.shape
        H, Dh = (Wq.shape[1], Wq.shape[2])
        M = mem0.shape[1]
        scale = Dh ** (-0.5)
        n_seg = S // seg_len
        L = M + seg_len
        idx = jnp.arange(L)
        mask = (idx[:, None] < M) | (idx[:, None] >= idx[None, :])
        mem = mem0
        outs = []
        for s in range(n_seg):
            xs = x[:, s * seg_len:(s + 1) * seg_len, :].copy()
            h = jnp.concatenate([mem, xs], axis=1)
            q = jnp.einsum('btd,dhe->bhte', h, Wq)
            k = jnp.einsum('btd,dhe->bhte', h, Wk)
            v = jnp.einsum('btd,dhe->bhte', h, Wv)
            scores = jnp.einsum('bhqe,bhke->bhqk', q, k) * scale
            scores = jnp.where(mask[None, None], scores, -1000000000.0)
            p = _softmax(scores, axis=-1)
            o = jnp.einsum('bhqk,bhke->bhqe', p, v)
            o = jnp.einsum('bhte,hed->btd', o, Wo)
            mem = o[:, :M, :].copy()
            outs.append(o[:, M:, :])
        return jnp.concatenate(outs, axis=1)

    def _B_ref(x, wqkv, w_phi, wo):
        B, S, D = x.shape
        H = 32
        Dh = D // H
        qkv = (lambda x, *d: x.transpose(*d))((x @ wqkv).reshape(B, S, 3, H, Dh), 2, 0, 3, 1, 4)
        q, k, v = (qkv[0], qkv[1], qkv[2])
        pq = jnp.einsum('bhsd,hdf->bhsf', q, w_phi)
        pk = jnp.einsum('bhsd,hdf->bhsf', k, w_phi)
        phi_q = jnp.concatenate([_softmax(pq, axis=-1), _softmax(-pq, axis=-1)], axis=-1)
        phi_k = jnp.concatenate([_softmax(pk, axis=-1), _softmax(-pk, axis=-1)], axis=-1)
        kv = jnp.einsum('bhsf,bhsd->bhfd', phi_k, v)
        z = jnp.einsum('bhsf->bhf', phi_k)
        num = jnp.einsum('bhqf,bhfd->bhqd', phi_q, kv)
        den = jnp.einsum('bhqf,bhf->bhq', phi_q, z)[..., None] + 1e-06
        o = num / den
        return (lambda x, *d: x.transpose(*d))(o, 0, 2, 1, 3).reshape(B, S, D) @ wo
    x = A_x
    x = x + _A_ref(_layernorm(x, axis=-1), A_mem0, A_Wq, A_Wk, A_Wv, A_Wo, A_seg_len)
    x = x + _B_ref(_layernorm(x, axis=-1), B_wqkv, B_w_phi, B_wo)
    x = x + _A_ref(_layernorm(x, axis=-1), A_mem0, A_Wq, A_Wk, A_Wv, A_Wo, A_seg_len)
    x = x + _B_ref(_layernorm(x, axis=-1), B_wqkv, B_w_phi, B_wo)
    return x
```

```python
import jax
import jax.numpy as jnp
from jax import lax
from jax.experimental import pallas as pl
from jax.experimental.pallas import tpu as pltpu

S, D = 2048, 640
AH, ADH, M, SEG = 32, 192, 8, 32
NP = AH // 2
PW = 2 * ADH
BH, BDH = 32, 20
NG, GH = 4, 8
GR = BDH * GH
TB = 256
bf16, f32, u32 = jnp.bfloat16, jnp.float32, jnp.uint32
SCALE = ADH ** -0.5
NEG = -1e9
JUNK = -1e30
NT = (((1,), (1,)), ((), ()))


def _layernorm(x):
    m = jnp.mean(x, axis=-1, keepdims=True)
    xc = x - m
    v = jnp.mean(xc * xc, axis=-1, keepdims=True)
    return xc * lax.rsqrt(v + 1e-5)


def _iota(shape, dim):
    return lax.broadcasted_iota(jnp.int32, shape, dim)


def _make_masks():
    r = _iota((48, 96), 0)
    c = _iota((48, 96), 1)
    c = jnp.where(c >= 48, c - 48, c)
    valid_a = c < 40
    keep_a = ((r < 8) | (r >= c)) & valid_a
    fill_a = jnp.where(valid_a, NEG, JUNK).astype(f32)
    lr = jnp.where(r < 16, r, jnp.where(r < 24, r - 16, r - 8))
    lc = jnp.where(c < 16, c, jnp.where(c < 24, c - 16, c - 8))
    valid_b = c >= 8
    keep_b = ((lr < 8) | (lr >= lc)) & valid_b
    fill_b = jnp.where(valid_b, NEG, JUNK).astype(f32)
    return keep_a, fill_a, keep_b, fill_b


def _blockdiag(k):
    ku = pltpu.bitcast(k, u32)
    lo = _iota(ku.shape, 1) < ADH
    z = jnp.zeros_like(ku)
    return pltpu.bitcast(jnp.concatenate([jnp.where(lo, ku, z), jnp.where(lo, z, ku)], axis=0), bf16)


def _attn_scores(q, k):
    return lax.dot_general(q, _blockdiag(k), NT, preferred_element_type=f32)


def _attn_softmax(s, keep, fill):
    s = jnp.where(keep, s * SCALE, fill)
    h0 = _iota((48, 96), 1) < 48
    m0 = jnp.max(jnp.where(h0, s, -jnp.inf), axis=-1, keepdims=True)
    m1 = jnp.max(jnp.where(h0, -jnp.inf, s), axis=-1, keepdims=True)
    e = jnp.exp(s - jnp.where(h0, m0, m1))
    l0 = jnp.sum(jnp.where(h0, e, 0.0), axis=-1, keepdims=True)
    l1 = jnp.sum(jnp.where(h0, 0.0, e), axis=-1, keepdims=True)
    return (e * jnp.where(h0, 1.0 / l0, 1.0 / l1)).astype(bf16)


def _features(p):
    t = p.shape[-1]
    p4 = p.reshape(NG, BDH, GH, t)
    mx = jnp.max(p4, axis=1, keepdims=True)
    mn = jnp.min(p4, axis=1, keepdims=True)
    ep = jnp.exp(p4 - mx)
    en = jnp.exp(mn - p4)
    pos = ep * (1.0 / jnp.sum(ep, axis=1, keepdims=True))
    neg = en * (1.0 / jnp.sum(en, axis=1, keepdims=True))
    return jnp.concatenate([pos, neg], axis=1).reshape(NG, 2 * GR, t)


def _kernel(x_hbm, mem_ref, wq_hbm, wk_hbm, wv_hbm, wo_hbm, bw_ref, wphi_ref, bwo_ref, o_ref,
            x_scr, sav_scr, wqkv_scr, wo_scr, wpt_scr, wvt_scr, bwo_scr, phiq_scr, kvt_scr, lhs2_scr,
            xin_scr, stage_scr, sems):
    w_hbm = (wq_hbm, wk_hbm, wv_hbm, wo_hbm)

    def w_copy(j, m):
        return pltpu.make_async_copy(w_hbm[m].at[pl.ds(j * PW, PW), :], stage_scr.at[m, j], sems.at[m, j])

    x_copy = pltpu.make_async_copy(x_hbm, xin_scr, sems.at[4, 0])
    x_copy.start()
    for j in range(NP):
        for m in range(4):
            w_copy(j, m).start()

    r = _iota((D, D), 0)
    c = _iota((D, D), 1)
    g_r, f_r, h_r = r // GR, (r % GR) // GH, r % GH
    head_r = g_r * GH + h_r
    same_head = head_r == c // BDH
    et = (_iota((D, BDH), 1) == (_iota((D, BDH), 0) % GR) // GH).astype(bf16)
    pm = lax.dot_general(et, wphi_ref[...], NT, preferred_element_type=f32)
    pm = jnp.where(same_head, pm, 0.0).astype(bf16)
    perm = (c == head_r * BDH + f_r).astype(bf16)
    wpt_scr[0:D] = lax.dot_general(pm, bw_ref[:, 0:D], NT, preferred_element_type=f32).astype(bf16)
    wpt_scr[D:2 * D] = lax.dot_general(pm, bw_ref[:, D:2 * D], NT, preferred_element_type=f32).astype(bf16)
    wvt_scr[...] = lax.dot_general(perm, bw_ref[:, 2 * D:3 * D], NT, preferred_element_type=f32).astype(bf16)
    bwo_scr[...] = jnp.dot(perm, bwo_ref[...], preferred_element_type=f32).astype(bf16)

    x_copy.wait()
    x_scr[...] = xin_scr[...].astype(f32)

    eye128 = (_iota((128, 128), 0) == _iota((128, 128), 1)).astype(bf16)

    def relayout(j, carry):
        for m in range(3):
            w_copy(j, m).wait()
            for t in range(D // 128):
                blk = stage_scr[m, j, :, t * 128:(t + 1) * 128]
                tr = lax.dot_general(eye128, blk, NT, preferred_element_type=f32)
                wqkv_scr[j, t * 64:(t + 1) * 64, m * PW:(m + 1) * PW] = pltpu.bitcast(tr.astype(bf16), u32)
        w_copy(j, 3).wait()
        wo_scr[j] = pltpu.bitcast(stage_scr[3, j], u32)
        return carry

    lax.fori_loop(0, NP, relayout, 0)

    def a_pass(h, keep, fill, pre, post):
        def qkv(j):
            w = pltpu.bitcast(wqkv_scr[j], bf16)
            return jnp.dot(h, w, preferred_element_type=f32).astype(bf16)

        def oproj(j, o):
            return jnp.dot(o, pltpu.bitcast(wo_scr[j], bf16), preferred_element_type=f32)

        rs = {0: qkv(0)}
        ws, ss, os_ = {}, {}, {}
        acc = None
        for j in range(NP + 2):
            if j < NP:
                ws[j] = pre(j, rs.pop(j))
                ss[j] = _attn_scores(ws[j][:, 0:PW], ws[j][:, PW:2 * PW])
            if j + 1 < NP:
                rs[j + 1] = qkv(j + 1)
            if 1 <= j <= NP:
                p = _attn_softmax(ss.pop(j - 1), keep, fill)
                vbd = _blockdiag(ws.pop(j - 1)[:, 2 * PW:3 * PW])
                o = jnp.dot(p, vbd, preferred_element_type=f32)
                os_[j - 1] = post(j - 1, o).astype(bf16)
            if j >= 2:
                t = oproj(j - 2, os_.pop(j - 2))
                acc = t if acc is None else acc + t
        return acc

    def a_layer():
        keep_a, fill_a, keep_b, fill_b = _make_masks()

        def step(it, mem):
            r0 = pl.multiple_of(it * 64, 64)
            xs = x_scr[pl.ds(r0, 64), :]
            xn = _layernorm(xs)
            h_a = jnp.concatenate([mem, xn[0:40]], axis=0).astype(bf16)
            osav = {}

            def pre_a(j, r):
                sav_scr[j] = r[32:48]
                return r

            def post_a(j, o):
                osav[j] = o[32:40]
                return o[0:32]

            acc_a = a_pass(h_a, keep_a, fill_a, pre_a, post_a)
            h_b = jnp.concatenate([acc_a[0:8], xn[40:64]], axis=0).astype(bf16)

            def pre_b(j, r):
                return jnp.concatenate([sav_scr[j], r], axis=0)

            def post_b(j, o):
                return jnp.concatenate([osav[j], o[8:48]], axis=0)

            acc_b = a_pass(h_b, keep_b, fill_b, pre_b, post_b)
            out = jnp.concatenate([acc_a[8:32], acc_b[0:16], acc_b[24:48]], axis=0)
            x_scr[pl.ds(r0, 64), :] = xs + out
            return acc_b[16:24]

        lax.fori_loop(0, S // 64, step, mem_ref[...].astype(f32))

    def b_layer():
        kvt_scr[...] = jnp.zeros_like(kvt_scr)
        ones = jnp.ones((16, TB), bf16)

        def pass1(i, carry):
            r0 = pl.multiple_of(i * TB, TB)
            xn = _layernorm(x_scr[pl.ds(r0, TB), :]).astype(bf16)
            pk = lax.dot_general(wpt_scr[D:2 * D], xn, NT, preferred_element_type=f32)
            vt = lax.dot_general(wvt_scr[...], xn, NT, preferred_element_type=f32).astype(bf16)
            pq = lax.dot_general(wpt_scr[0:D], xn, NT, preferred_element_type=f32)
            phik = _features(pk).astype(bf16)
            for g in range(NG):
                lhs = jnp.concatenate([vt[g * GR:(g + 1) * GR], ones], axis=0)
                kvt_scr[g] += lax.dot_general(lhs, phik[g], NT, preferred_element_type=f32)
            phiq_scr[i] = _features(pq).astype(bf16)
            return carry

        lax.fori_loop(0, S // TB, pass1, 0)

        rr = _iota((GR + 16, 2 * GR), 0)
        cc = _iota((GR + 16, 2 * GR), 1)
        m2 = ((rr % GH) == (cc % GH)) & (rr < GR + GH)
        for g in range(NG):
            kv = kvt_scr[g]
            src = jnp.concatenate([kv[0:GR], jnp.broadcast_to(kv[GR:GR + 1], (16, 2 * GR))], axis=0)
            lhs2_scr[g] = jnp.where(m2, src, 0.0).astype(bf16)

        eye = (_iota((128, 128), 0) == _iota((128, 128), 1)).astype(bf16)

        def pass2(i, carry):
            r0 = pl.multiple_of(i * TB, TB)
            ots = []
            for g in range(NG):
                res = jnp.dot(lhs2_scr[g], phiq_scr[i, g], preferred_element_type=f32)
                inv = 1.0 / (res[GR:GR + GH] + 1e-6)
                ots.append((res[0:GR].reshape(BDH, GH, TB) * inv[None]).reshape(GR, TB))
            ot = jnp.concatenate(ots, axis=0).astype(bf16)
            o = jnp.concatenate(
                [lax.dot_general(eye, ot[:, t * 128:(t + 1) * 128], NT, preferred_element_type=f32)
                 for t in range(TB // 128)], axis=0).astype(bf16)
            x_scr[pl.ds(r0, TB), :] += jnp.dot(o, bwo_scr[...], preferred_element_type=f32)
            return carry

        lax.fori_loop(0, S // TB, pass2, 0)

    def layer(_, carry):
        a_layer()
        b_layer()
        return carry

    lax.fori_loop(0, 2, layer, 0)
    o_ref[...] = x_scr[...].astype(bf16)


@jax.jit
def pallas_interleave_layers__memory_aug_recurrent_mem_tr__linear_kernel_hedgehog__prompt_kernel(A_x, A_mem0, A_Wq, A_Wk, A_Wv, A_Wo, A_seg_len, B_x, B_wqkv, B_w_phi, B_wo):
    def tr(w):
        return w.transpose(1, 2, 0).reshape(AH * ADH, D)
    any_spec = pl.BlockSpec(memory_space=pl.ANY)
    vmem_spec = pl.BlockSpec(memory_space=pltpu.VMEM)
    out = pl.pallas_call(
        _kernel,
        out_shape=jax.ShapeDtypeStruct((S, D), bf16),
        in_specs=[any_spec, vmem_spec, any_spec, any_spec, any_spec, any_spec, vmem_spec, vmem_spec, vmem_spec],
        scratch_shapes=[
            pltpu.VMEM((S, D), f32),
            pltpu.VMEM((NP, 16, 3 * PW), bf16),
            pltpu.VMEM((NP, D // 2, 3 * PW), u32),
            pltpu.VMEM((NP, PW // 2, D), u32),
            pltpu.VMEM((2 * D, D), bf16),
            pltpu.VMEM((D, D), bf16),
            pltpu.VMEM((D, D), bf16),
            pltpu.VMEM((S // TB, NG, 2 * GR, TB), bf16),
            pltpu.VMEM((NG, GR + 16, 2 * GR), f32),
            pltpu.VMEM((NG, GR + 16, 2 * GR), bf16),
            pltpu.VMEM((S, D), bf16),
            pltpu.VMEM((4, NP, PW, D), bf16),
            pltpu.SemaphoreType.DMA((5, NP)),
        ],
        name="fused_layers",
        compiler_params=pltpu.CompilerParams(vmem_limit_bytes=126 * 1024 * 1024),
    )(A_x.reshape(S, D), A_mem0.reshape(M, D), tr(A_Wq), tr(A_Wk), tr(A_Wv), A_Wo.reshape(AH * ADH, D),
      B_wqkv, B_w_phi.reshape(D, BDH), B_wo)
    return out.reshape(1, S, D)
```

```python
import functools
import jax
import jax.numpy as jnp
from jax import lax
from jax.experimental import pallas as pl
from jax.experimental.pallas import tpu as pltpu

S, D = 2048, 640
AH, ADH, M, SEG = 32, 192, 8, 32
NP = AH // 2
PW = 2 * ADH
BH, BDH = 32, 20
NG = BH // 2
GR = 2 * BDH
TB = 256
NB = S // TB
bf16, f32, u32 = jnp.bfloat16, jnp.float32, jnp.uint32
SCALE = ADH ** -0.5
NEG = -1e9
JUNK = -1e30
NT = (((1,), (1,)), ((), ()))


def _layernorm(x):
    m = jnp.mean(x, axis=-1, keepdims=True)
    xc = x - m
    v = jnp.mean(xc * xc, axis=-1, keepdims=True)
    return xc * lax.rsqrt(v + 1e-5)


def _iota(shape, dim):
    return lax.broadcasted_iota(jnp.int32, shape, dim)


def _make_masks():
    r = _iota((48, 96), 0)
    c = _iota((48, 96), 1)
    c = jnp.where(c >= 48, c - 48, c)
    valid_a = c < 40
    keep_a = ((r < 8) | (r >= c)) & valid_a
    fill_a = jnp.where(valid_a, NEG, JUNK).astype(f32)
    lr = jnp.where(r < 16, r, jnp.where(r < 24, r - 16, r - 8))
    lc = jnp.where(c < 16, c, jnp.where(c < 24, c - 16, c - 8))
    valid_b = c >= 8
    keep_b = ((lr < 8) | (lr >= lc)) & valid_b
    fill_b = jnp.where(valid_b, NEG, JUNK).astype(f32)
    return keep_a, fill_a, keep_b, fill_b


def _blockdiag(k):
    ku = pltpu.bitcast(k, u32)
    lo = _iota(ku.shape, 1) < ADH
    z = jnp.zeros_like(ku)
    return pltpu.bitcast(jnp.concatenate([jnp.where(lo, ku, z), jnp.where(lo, z, ku)], axis=0), bf16)


def _attn_scores(q, k):
    return lax.dot_general(q, _blockdiag(k), NT, preferred_element_type=f32)


def _attn_softmax(s, keep, fill):
    s = jnp.where(keep, s * SCALE, fill)
    h0 = _iota((48, 96), 1) < 48
    m0 = jnp.max(jnp.where(h0, s, -jnp.inf), axis=-1, keepdims=True)
    m1 = jnp.max(jnp.where(h0, -jnp.inf, s), axis=-1, keepdims=True)
    e = jnp.exp(s - jnp.where(h0, m0, m1))
    l0 = jnp.sum(jnp.where(h0, e, 0.0), axis=-1, keepdims=True)
    l1 = jnp.sum(jnp.where(h0, 0.0, e), axis=-1, keepdims=True)
    return (e * jnp.where(h0, 1.0 / l0, 1.0 / l1)).astype(bf16)


def _pair_reduce(op, a):
    a = op(a, pltpu.roll(a, 2, 1))
    return op(a, pltpu.roll(a, 4, 1))


def _features(p):
    t = p.shape[-1]
    ng = p.shape[0] // GR
    p4 = p.reshape(ng, 5, 8, t)
    mx = _pair_reduce(jnp.maximum, jnp.max(p4, axis=1))[:, None]
    mn = _pair_reduce(jnp.minimum, jnp.min(p4, axis=1))[:, None]
    ep = jnp.exp(p4 - mx)
    en = jnp.exp(mn - p4)
    pos = ep * (1.0 / _pair_reduce(jnp.add, jnp.sum(ep, axis=1)))[:, None]
    neg = en * (1.0 / _pair_reduce(jnp.add, jnp.sum(en, axis=1)))[:, None]
    return jnp.concatenate([pos, neg], axis=1).reshape(ng, 2 * GR, t).astype(bf16)


def _kernel(x_hbm, mem_ref, wq_hbm, wk_hbm, wv_hbm, wo_hbm, bw_hbm, wphi_ref, bwo_hbm, o_hbm,
            x_scr, sav_scr, wqkv_scr, wo_scr, wb_scr, bw_scr, bwo_scr, phiq_scr, kvt_scr, lhs2_scr,
            xin_scr, stage_scr, xpre_scr, hpre_scr, pre_scr, xnb_scr, o_scr, sems, *, opt):
    n_pre = opt.get("n_pre", 17)
    w_hbm = tuple(w.bitcast(u32) for w in (wq_hbm, wk_hbm, wv_hbm, wo_hbm))

    def w_copy(j, m):
        dst = wo_scr.at[j] if m == 3 else stage_scr.at[m, j]
        r0 = j * (PW // 2) if isinstance(j, int) else pl.multiple_of(j * (PW // 2), PW // 2)
        return pltpu.make_async_copy(w_hbm[m].at[pl.ds(r0, PW // 2), :], dst, sems.at[m, j])

    def out_copy(i):
        return pltpu.make_async_copy(xin_scr.at[pl.ds(i * TB, TB), :], o_hbm.at[pl.ds(i * TB, TB), :],
                                     sems.at[5, i])

    def xpre_copy(it):
        return pltpu.make_async_copy(x_hbm.at[pl.ds(pl.multiple_of(it * 64, 64) + 24, 16), :],
                                     xpre_scr.at[pl.ds(pl.multiple_of(it * 16, 16), 16), :], sems.at[4, 3])

    def xstep_copy(it):
        r0 = it * 64 if isinstance(it, int) else pl.multiple_of(it * 64, 64)
        return pltpu.make_async_copy(x_hbm.at[pl.ds(r0, 64), :], xin_scr.at[pl.ds(r0, 64), :],
                                     sems.at[6 + it // NP, it % NP])

    xr0 = n_pre * 64
    xrest_copy = pltpu.make_async_copy(x_hbm.at[pl.ds(xr0, S - xr0), :], xin_scr.at[pl.ds(xr0, S - xr0), :],
                                       sems.at[4, 0])
    bw_copy = pltpu.make_async_copy(bw_hbm.bitcast(u32), bw_scr, sems.at[4, 1])
    bwo_copy = pltpu.make_async_copy(bwo_hbm.bitcast(u32), bwo_scr, sems.at[4, 2])
    def loop(lo, hi, fn):
        lax.fori_loop(lo, hi, lambda i, c: (fn(i), c)[1], 0)

    def start_qkv(j):
        for m in range(3):
            w_copy(j, m).start()

    loop(0, n_pre, lambda it: xpre_copy(it).start())
    fold_late = opt.get("fold_late", True)
    start_qkv(0)
    if not fold_late:
        bw_copy.start()
    loop(1, NP, start_qkv)
    if fold_late:
        bw_copy.start()
    loop(0, NP, lambda j: w_copy(j, 3).start())
    loop(0, n_pre, lambda it: xstep_copy(it).start())
    xrest_copy.start()
    bwo_copy.start()

    x_scr[0:128, :] = jnp.zeros((128, D), f32)
    loop(0, n_pre, lambda it: xpre_copy(it).wait())

    def hpre_ln(it):
        rows = pl.ds(pl.multiple_of(it * 16, 16), 16)
        hpre_scr[rows, :] = _layernorm(xpre_scr[rows, :].astype(f32)).astype(bf16)

    if opt.get("ln_loop", False):
        loop(0, n_pre, hpre_ln)
    else:
        hpre_scr[...] = _layernorm(xpre_scr[...].astype(f32)).astype(bf16)

    def relayout_tile(j, m, t):
        lanes = pl.ds(t * 128, 128) if isinstance(t, int) else pl.ds(pl.multiple_of(t * 128, 128), 128)
        rows = pl.ds(t * 64, 64) if isinstance(t, int) else pl.ds(pl.multiple_of(t * 64, 64), 64)
        blk = pltpu.bitcast(stage_scr[m, j, :, lanes], bf16)
        wqkv_scr[j, rows, m * PW:(m + 1) * PW] = pltpu.bitcast(blk.T, u32)

    def pre_qkv(j):
        pre_scr[j] = jnp.dot(hpre_scr[...], pltpu.bitcast(wqkv_scr[j], bf16),
                             preferred_element_type=f32).astype(bf16)

    def relayout_step(j):
        for m in range(3):
            w_copy(j, m).wait()
        pre_qkv(j - 1)
        for m in range(3):
            for t in range(D // 128):
                relayout_tile(j, m, t)

    def fold_b_weights(t):
        lo = pl.multiple_of(128 * jnp.clip(t - 1, 0, 2), 128)
        r = 128 * t + _iota((128, 384), 0)
        c = lo + _iota((128, 384), 1)
        same_head = 2 * (r // GR) + r % 2 == c // BDH
        rf = (128 * t + _iota((128, BDH), 0)) % GR
        et = (_iota((128, BDH), 1) == 4 * (rf // 8) + (rf % 8) // 2).astype(bf16)
        pm = lax.dot_general(et, wphi_ref[pl.ds(lo, 384), :], NT, preferred_element_type=f32)
        pm = jnp.where(same_head, pm, 0.0).astype(bf16)
        rows = pl.ds(pl.multiple_of(t * 64, 64), 64)
        for m in range(2):
            w = pltpu.bitcast(bw_scr[:, pl.ds(pl.multiple_of(m * D + lo, 128), 384)], bf16)
            wb_scr[m, rows, :] = pltpu.bitcast(
                lax.dot_general(pm, w, NT, preferred_element_type=f32).astype(bf16), u32)
        w = pltpu.bitcast(bw_scr[:, pl.ds(pl.multiple_of(2 * D + 128 * t, 128), 128)], bf16)
        wb_scr[2, rows, :] = pltpu.bitcast(w.T, u32)

    for m in range(3):
        w_copy(0, m).wait()
    if opt.get("r0_loop", False):
        loop(0, D // 128, lambda t: [relayout_tile(0, m, t) for m in range(3)])
    else:
        for m in range(3):
            for t in range(D // 128):
                relayout_tile(0, m, t)
    if not fold_late:
        bw_copy.wait()
        loop(0, D // 128, fold_b_weights)
    loop(1, NP, relayout_step)
    pre_qkv(NP - 1)
    if fold_late:
        bw_copy.wait()
        loop(0, D // 128, fold_b_weights)
    loop(0, NP, lambda j: w_copy(j, 3).wait())

    HB = NG // 2
    ones = jnp.ones((HB, 8, 128), f32)

    def b1_w(m, h):
        r0 = h * 160 if isinstance(h, int) else pl.multiple_of(h * 160, 160)
        return pltpu.bitcast(wb_scr[m, pl.ds(r0, 160), :], bf16)

    def b1_pk(h, xn):
        pk = lax.dot_general(b1_w(1, h), xn, NT, preferred_element_type=f32)
        return _features(pk)

    def b1_v(h, xn):
        vt = lax.dot_general(b1_w(2, h), xn, NT, preferred_element_type=f32)
        return jnp.concatenate([vt.reshape(HB, GR, 128), ones], axis=1).astype(bf16)

    def b1_pq(b, h, xn):
        pq = lax.dot_general(b1_w(0, h), xn, NT, preferred_element_type=f32)
        phiq_scr[b, pl.ds(pl.multiple_of(h * HB, HB), HB)] = _features(pq)

    def b1_kvt(h, valid, phik, lhs):
        for g in range(HB):
            t = lax.dot_general(lhs[g], phik[g], NT, preferred_element_type=f32)
            if valid is not None:
                t = jnp.where(valid, t, 0.0)
            kvt_scr[h * HB + g] += t

    def store_xnb(slot, val):
        xnb_scr[slot] = val

    def b1_ln(b):
        return _layernorm(x_scr[pl.ds(pl.multiple_of(b * 128, 128), 128), :]).astype(bf16)

    def a_pass(h, keep, fill, pre, post, hooks):
        def qkv(j):
            w = pltpu.bitcast(wqkv_scr[j], bf16)
            return jnp.dot(h, w, preferred_element_type=f32).astype(bf16)

        def oproj(j, o):
            return jnp.dot(o, pltpu.bitcast(wo_scr[j], bf16), preferred_element_type=f32)

        lag = dict(Q=0, S=opt.get("lagS", 1), P=opt.get("lagP", 3), O=opt.get("lagO", 4))
        order = opt.get("order", "QSPO")
        rs, ws, ss, os_ = {}, {}, {}, {}
        acc = None
        for i in range(NP + max(lag.values())):
            for fn in hooks.get(i, ()):
                fn()
            for op in order:
                j = i - lag[op]
                if not (0 <= j < NP):
                    continue
                if op == "Q":
                    rs[j] = qkv(j)
                elif op == "S":
                    ws[j] = pre(j, rs.pop(j))
                    ss[j] = _attn_scores(ws[j][:, 0:PW], ws[j][:, PW:2 * PW])
                elif op == "P":
                    p = _attn_softmax(ss.pop(j), keep, fill)
                    vbd = _blockdiag(ws.pop(j)[:, 2 * PW:3 * PW])
                    o = jnp.dot(p, vbd, preferred_element_type=f32)
                    os_[j] = post(j, o).astype(bf16)
                else:
                    t = oproj(j, os_.pop(j))
                    acc = t if acc is None else acc + t
        for fn in hooks.get(NP + max(lag.values()), ()):
            fn()
        return acc

    def a_layer(l):
        keep_a, fill_a, keep_b, fill_b = _make_masks()
        kvt_scr[...] = jnp.zeros_like(kvt_scr)
        xnb_scr[0] = b1_ln(0)
        pos = opt.get("pos", dict(K=("a", 0), V=("b", 0), Q=("a", 17), T=("b", 8), L=("b", 4)))

        def step(use_pre, it, mem):
            r0 = pl.multiple_of(it * 64, 64)
            if use_pre:
                xstep_copy(it).wait()
                xs = xin_scr[pl.ds(r0, 64), :].astype(f32)
            else:
                xs = x_scr[pl.ds(r0, 64), :]
            xn = _layernorm(xs)
            h_a = jnp.concatenate([mem, xn[0:24] if use_pre else xn[0:40]], axis=0).astype(bf16)
            osav = {}

            hb = jnp.maximum(it - 3, 0)
            fb, fh, valid = hb // 2, hb % 2, it >= 3
            st = {}
            fillers = dict(
                K=lambda: st.update(phik=b1_pk(fh, xnb_scr[it % 2])),
                V=lambda: st.update(lhs=b1_v(fh, xnb_scr[it % 2])),
                Q=lambda: b1_pq(fb, fh, xnb_scr[it % 2]),
                T=lambda: b1_kvt(fh, valid, st["phik"], st["lhs"]),
                L=lambda: store_xnb((it + 1) % 2, b1_ln(jnp.maximum(it - 2, 0) // 2)),
            )
            hooks = {"a": {}, "b": {}}
            if opt.get("fuse", True):
                for name, (ps, slot) in pos.items():
                    hooks[ps].setdefault(slot, []).append(fillers[name])

            def pre_a(j, r):
                if use_pre:
                    sv = pre_scr[j, pl.ds(pl.multiple_of(it * 16, 16), 16), :]
                    sav_scr[j] = sv
                    return jnp.concatenate([r, sv], axis=0)
                sav_scr[j] = r[32:48]
                return r

            def post_a(j, o):
                osav[j] = o[32:40]
                return o[0:32]

            acc_a = a_pass(h_a, keep_a, fill_a, pre_a, post_a, hooks["a"])
            h_b = jnp.concatenate([acc_a[0:8], xn[40:64]], axis=0).astype(bf16)

            def pre_b(j, r):
                return jnp.concatenate([sav_scr[j], r], axis=0)

            def post_b(j, o):
                return jnp.concatenate([osav[j], o[8:48]], axis=0)

            acc_b = a_pass(h_b, keep_b, fill_b, pre_b, post_b, hooks["b"])
            out = jnp.concatenate([acc_a[8:32], acc_b[0:16], acc_b[24:48]], axis=0)
            x_scr[pl.ds(r0, 64), :] = xs + out
            return acc_b[16:24]

        n_var = jnp.where(l == 0, n_pre, 0)
        mem = lax.fori_loop(0, n_var, functools.partial(step, True), mem_ref[...].astype(f32))

        @pl.when(l == 0)
        def _():
            xrest_copy.wait()

            def cast(it, c):
                rows = pl.ds(pl.multiple_of(it * 64, 64), 64)
                x_scr[rows, :] = xin_scr[rows, :].astype(f32)
                return c

            lax.fori_loop(n_pre, S // 64, cast, 0)
            bwo_copy.wait()
            for i in range(NB):
                out_copy(i).start()

        lax.fori_loop(n_var, S // 64, functools.partial(step, False), mem)

    def b_layer():
        for i in range(NB):
            out_copy(i).wait()

        first = 29 if opt.get("fuse", True) else 0
        if first:
            todo = [(hb // 2, hb % 2) for hb in range(first, 32)]
            xns = {b: b1_ln(b) for b in sorted({b for b, _ in todo})}
            pend = None
            for b, h in todo:
                phik = b1_pk(h, xns[b])
                if pend is not None:
                    b1_kvt(*pend)
                lhs = b1_v(h, xns[b])
                b1_pq(b, h, xns[b])
                pend = (h, None, phik, lhs)
            b1_kvt(*pend)
        else:
            def p1(hb, c):
                b, h = hb // 2, hb % 2
                xn = b1_ln(b)
                phik = b1_pk(h, xn)
                lhs = b1_v(h, xn)
                b1_pq(b, h, xn)
                b1_kvt(h, None, phik, lhs)
                return c
            lax.fori_loop(0, 32, p1, 0)

        rr = _iota((GR + 8, 2 * GR), 0)
        cc = _iota((GR + 8, 2 * GR), 1)
        m2 = jnp.where(rr < GR, rr // BDH, (rr - GR) // 4) == cc % 2
        for g in range(NG):
            lhs2_scr[g] = jnp.where(m2, kvt_scr[g], 0.0).astype(bf16)

        lo4 = _iota((8, TB), 0) < 4

        def numden(i):
            outs = []
            for g in range(NG):
                phiq = jnp.concatenate([phiq_scr[2 * i, g], phiq_scr[2 * i + 1, g]], axis=1)
                res = jnp.dot(lhs2_scr[g], phiq, preferred_element_type=f32)
                inv = 1.0 / (res[GR:GR + 8] + 1e-6)
                swp = pltpu.roll(inv, 4, 0)
                i0 = jnp.where(lo4, inv, swp)
                i1 = jnp.where(lo4, swp, inv)
                outs += [res[0:8] * i0, res[8:16] * i0, res[16:24] * inv, res[24:32] * i1, res[32:40] * i1]
            return jnp.concatenate(outs, axis=0).T.astype(bf16)

        def proj(i, o):
            rows = pl.ds(i * TB, TB) if isinstance(i, int) else pl.ds(pl.multiple_of(i * TB, TB), TB)
            xnew = x_scr[rows, :] + jnp.dot(o, pltpu.bitcast(bwo_scr[...], bf16), preferred_element_type=f32)
            x_scr[rows, :] = xnew
            xin_scr[rows, :] = xnew.astype(bf16)
            out_copy(i).start()

        if opt.get("p2pipe", True):
            o_scr[0] = numden(0)

            def pass2(i, carry):
                o_next = numden(i + 1)
                proj(i, o_scr[i % 2])
                o_scr[(i + 1) % 2] = o_next
                return carry

            lax.fori_loop(0, NB - 1, pass2, 0)
            proj(NB - 1, o_scr[(NB - 1) % 2])
        else:
            lax.fori_loop(0, NB, lambda i, c: (proj(i, numden(i)), c)[1], 0)

    def layer(l, carry):
        if opt.get("A", True):
            a_layer(l)
        else:
            @pl.when(l == 0)
            def _():
                for it in range(n_pre):
                    xstep_copy(it).wait()
                xrest_copy.wait()
                x_scr[...] = xin_scr[...].astype(f32)
                bwo_copy.wait()
                for i in range(NB):
                    out_copy(i).start()
        if opt.get("B", True):
            b_layer()
        return carry

    lax.fori_loop(0, 2, layer, 0)
    if not opt.get("B", True):
        for i in range(NB):
            out_copy(i).wait()
            xin_scr[i * TB:(i + 1) * TB, :] = x_scr[i * TB:(i + 1) * TB, :].astype(bf16)
            out_copy(i).start()
    for i in range(NB):
        out_copy(i).wait()


opt = {}
n_pre = opt.get("n_pre", 17)

@jax.jit
def pallas_interleave_layers__memory_aug_recurrent_mem_tr__linear_kernel_hedgehog__prompt_kernel(A_x, A_mem0, A_Wq, A_Wk, A_Wv, A_Wo, A_seg_len, B_x, B_wqkv, B_w_phi, B_wo):
    def tr(w):
        return w.transpose(1, 2, 0).reshape(AH * ADH, D)
    any_spec = pl.BlockSpec(memory_space=pl.ANY)
    vmem_spec = pl.BlockSpec(memory_space=pltpu.VMEM)
    out = pl.pallas_call(
        functools.partial(_kernel, opt=opt),
        out_shape=jax.ShapeDtypeStruct((S, D), bf16),
        in_specs=[any_spec, vmem_spec, any_spec, any_spec, any_spec, any_spec, any_spec, vmem_spec, any_spec],
        out_specs=any_spec,
        scratch_shapes=[
            pltpu.VMEM((S, D), f32),
            pltpu.VMEM((NP, 16, 3 * PW), bf16),
            pltpu.VMEM((NP, D // 2, 3 * PW), u32),
            pltpu.VMEM((NP, PW // 2, D), u32),
            pltpu.VMEM((3, D // 2, D), u32),
            pltpu.VMEM((D // 2, 3 * D), u32),
            pltpu.VMEM((D // 2, D), u32),
            pltpu.VMEM((S // 128, NG, 2 * GR, 128), bf16),
            pltpu.VMEM((NG, GR + 8, 2 * GR), f32),
            pltpu.VMEM((NG, GR + 8, 2 * GR), bf16),
            pltpu.VMEM((S, D), bf16),
            pltpu.VMEM((3, NP, PW // 2, D), u32),
            pltpu.VMEM((max(n_pre, 1) * 16, D), bf16),
            pltpu.VMEM((max(n_pre, 1) * 16, D), bf16),
            pltpu.VMEM((NP, max(n_pre, 1) * 16, 3 * PW), bf16),
            pltpu.VMEM((2, 128, D), bf16),
            pltpu.VMEM((2, TB, D), bf16),
            pltpu.SemaphoreType.DMA((8, NP)),
        ],
        name="fused_layers",
        compiler_params=pltpu.CompilerParams(vmem_limit_bytes=126 * 1024 * 1024),
    )(A_x.reshape(S, D), A_mem0.reshape(M, D), tr(A_Wq), tr(A_Wk), tr(A_Wv), A_Wo.reshape(AH * ADH, D),
      B_wqkv, B_w_phi.reshape(D, BDH), B_wo)
    return out.reshape(1, S, D)
```

```python
import functools
import jax
import jax.numpy as jnp
from jax import lax
from jax.experimental import pallas as pl
from jax.experimental.pallas import tpu as pltpu

S, D = 2048, 640
AH, ADH, M, SEG = 32, 192, 8, 32
NP = AH // 2
PW = 2 * ADH
BH, BDH = 32, 20
NG = BH // 2
GR = 2 * BDH
TB = 256
NB = S // TB
bf16, f32, u32 = jnp.bfloat16, jnp.float32, jnp.uint32
SCALE = ADH ** -0.5
NEG = -1e9
JUNK = -1e30
NT = (((1,), (1,)), ((), ()))


def _layernorm(x):
    m = jnp.mean(x, axis=-1, keepdims=True)
    xc = x - m
    v = jnp.mean(xc * xc, axis=-1, keepdims=True)
    return xc * lax.rsqrt(v + 1e-5)


def _iota(shape, dim):
    return lax.broadcasted_iota(jnp.int32, shape, dim)


def _make_masks():
    r = _iota((48, 96), 0)
    c = _iota((48, 96), 1)
    c = jnp.where(c >= 48, c - 48, c)
    valid_a = c < 40
    keep_a = ((r < 8) | (r >= c)) & valid_a
    fill_a = jnp.where(valid_a, NEG, JUNK).astype(f32)
    lr = jnp.where(r < 16, r, jnp.where(r < 24, r - 16, r - 8))
    lc = jnp.where(c < 16, c, jnp.where(c < 24, c - 16, c - 8))
    valid_b = c >= 8
    keep_b = ((lr < 8) | (lr >= lc)) & valid_b
    fill_b = jnp.where(valid_b, NEG, JUNK).astype(f32)
    return keep_a, fill_a, keep_b, fill_b


def _blockdiag(k):
    ku = pltpu.bitcast(k, u32)
    lo = _iota(ku.shape, 1) < ADH
    z = jnp.zeros_like(ku)
    return pltpu.bitcast(jnp.concatenate([jnp.where(lo, ku, z), jnp.where(lo, z, ku)], axis=0), bf16)


def _attn_scores(q, k):
    return lax.dot_general(q, _blockdiag(k), NT, preferred_element_type=f32)


def _attn_softmax(s, keep, fill):
    s = jnp.where(keep, s * SCALE, fill)
    h0 = _iota((48, 96), 1) < 48
    m0 = jnp.max(jnp.where(h0, s, -jnp.inf), axis=-1, keepdims=True)
    m1 = jnp.max(jnp.where(h0, -jnp.inf, s), axis=-1, keepdims=True)
    e = jnp.exp(s - jnp.where(h0, m0, m1))
    l0 = jnp.sum(jnp.where(h0, e, 0.0), axis=-1, keepdims=True)
    l1 = jnp.sum(jnp.where(h0, 0.0, e), axis=-1, keepdims=True)
    return (e * jnp.where(h0, 1.0 / l0, 1.0 / l1)).astype(bf16)


def _pair_reduce(op, a):
    a = op(a, pltpu.roll(a, 2, 1))
    return op(a, pltpu.roll(a, 4, 1))


def _features(p):
    t = p.shape[-1]
    ng = p.shape[0] // GR
    p4 = p.reshape(ng, 5, 8, t)
    mx = _pair_reduce(jnp.maximum, jnp.max(p4, axis=1))[:, None]
    mn = _pair_reduce(jnp.minimum, jnp.min(p4, axis=1))[:, None]
    ep = jnp.exp(p4 - mx)
    en = jnp.exp(mn - p4)
    pos = ep * (1.0 / _pair_reduce(jnp.add, jnp.sum(ep, axis=1)))[:, None]
    neg = en * (1.0 / _pair_reduce(jnp.add, jnp.sum(en, axis=1)))[:, None]
    return jnp.concatenate([pos, neg], axis=1).reshape(ng, 2 * GR, t).astype(bf16)


def _kernel(x_hbm, x3_hbm, mem_hbm, wq_hbm, wk_hbm, wv_hbm, wo_hbm, bw_hbm, wphi_hbm, bwo_hbm, o_hbm,
            x_scr, sav_scr, wqkv_scr, wo_scr, wb_scr, bw_scr, bwo_scr, phiq_scr, kvt_scr, lhs2_scr,
            xin_scr, stage_scr, xpre_scr, hpre_scr, pre_scr, xnb_scr, o_scr, wphi_scr, mem_ref, wphi_ref, lhs_scr, sems, *, opt):
    n_pre = S // 64
    PC = opt.get("PC", 768)
    w_hbm = tuple(w.bitcast(u32) for w in (wq_hbm, wk_hbm, wv_hbm, wo_hbm))

    def w_copy(j, m):
        dst = wo_scr.at[j] if m == 3 else stage_scr.at[m, j]
        r0 = j * (PW // 2) if isinstance(j, int) else pl.multiple_of(j * (PW // 2), PW // 2)
        return pltpu.make_async_copy(w_hbm[m].at[pl.ds(r0, PW // 2), :], dst, sems.at[m, j])

    def w_piece(j, m, p, n):
        rows = PW // 2 // n
        return pltpu.make_async_copy(w_hbm[m].at[pl.ds(j * (PW // 2) + p * rows, rows), :],
                                     stage_scr.at[m, j, pl.ds(p * rows, rows), :], sems.at[m, j])

    def out_copy(i):
        return pltpu.make_async_copy(xin_scr.at[pl.ds(i * TB, TB), :], o_hbm.at[pl.ds(i * TB, TB), :],
                                     sems.at[5, i])

    NXP = 4

    def xpre_copy(q):
        steps = pl.ds(q * (n_pre // NXP), n_pre // NXP)
        return pltpu.make_async_copy(x3_hbm.at[steps, pl.ds(24, 16), :], xpre_scr.at[steps], sems.at[6, q])

    nx0 = opt.get("nx0", 2)
    x_first = pltpu.make_async_copy(x_hbm.at[pl.ds(0, nx0 * 64), :], xin_scr.at[pl.ds(0, nx0 * 64), :], sems.at[7, 0])
    x_rest = pltpu.make_async_copy(x_hbm.at[pl.ds(nx0 * 64, S - nx0 * 64), :],
                                   xin_scr.at[pl.ds(nx0 * 64, S - nx0 * 64), :], sems.at[7, 1])

    bw_copy = pltpu.make_async_copy(bw_hbm.bitcast(u32), bw_scr, sems.at[4, 1])
    bwo_copy = pltpu.make_async_copy(bwo_hbm.bitcast(u32), bwo_scr, sems.at[4, 2])
    mem_copy = pltpu.make_async_copy(mem_hbm, mem_ref, sems.at[4, 4])
    wphi_copy = pltpu.make_async_copy(wphi_hbm, wphi_ref, sems.at[4, 5])

    def loop(lo, hi, fn):
        lax.fori_loop(lo, hi, lambda i, c: (fn(i), c)[1], 0)

    def start_qkv(j):
        for m in range(3):
            w_copy(j, m).start()

    win = opt.get("win", 4)

    bwslot, woslot = opt.get("bwslot", 0), opt.get("woslot", 1)

    def start_wo():
        loop(0, NP, lambda j: w_copy(j, 3).start())

    def start_x():
        x_rest.start()
        bwo_copy.start()

    split = opt.get("split", (1,))
    for m in range(3):
        for p in range(split[0]):
            w_piece(0, m, p, split[0]).start()
    for q in range(NXP):
        xpre_copy(q).start()
    for j in range(1, len(split)):
        for m in range(3):
            for p in range(split[j]):
                w_piece(j, m, p, split[j]).start()
    mem_copy.start()
    wphi_copy.start()
    n_up = opt.get("n_up", win)
    later = list(range(n_up, win))
    if n_up > 1:
        loop(len(split), n_up, start_qkv)
    x_first.start()

    x_scr[0:128, :] = jnp.zeros((128, D), f32)
    xnb_scr[0] = jnp.zeros((128, D), bf16)
    wphi_copy.wait()
    mem_copy.wait()
    if opt.get("wphi3", True):
        for e in range(BDH):
            wphi_scr[pl.ds(e, BH, stride=BDH), :] = wphi_ref[e].astype(f32).T
    if later:
        start_qkv(later.pop(0))

    def hpre_chunk(q):
        xpre_copy(q).wait()
        xq = xpre_scr[pl.ds(q * (n_pre // NXP), n_pre // NXP)].reshape(128, D).astype(f32)
        hpre_scr[pl.ds(pl.multiple_of(q * 128, 128), 128), :] = _layernorm(xq).astype(bf16)

    if not opt.get("lnmerge", False):
        loop(0, NXP, hpre_chunk)
    if later:
        start_qkv(later.pop(0))

    def relayout_tile(j, m, t):
        lanes = pl.ds(t * 128, 128) if isinstance(t, int) else pl.ds(pl.multiple_of(t * 128, 128), 128)
        rows = pl.ds(t * 64, 64) if isinstance(t, int) else pl.ds(pl.multiple_of(t * 64, 64), 64)
        blk = pltpu.bitcast(stage_scr[m, j, :, lanes], bf16)
        wqkv_scr[j, rows, m * PW:(m + 1) * PW] = pltpu.bitcast(blk.T, u32)

    def pre_qkv(j):
        nch = opt.get("nch", 1)
        for c in range(nch):
            rows = pl.ds(c * (n_pre * 16 // nch), n_pre * 16 // nch)
            pre_scr[j, rows, :] = jnp.dot(hpre_scr[rows, :], pltpu.bitcast(wqkv_scr[j, :, 0:PC], bf16),
                                          preferred_element_type=f32).astype(bf16)

    def request(j):
        pl.when(j < NP)(lambda: [w_copy(j, m).wait() for m in range(3)] and None)
        nxt = j + win - 1
        pl.when(nxt < NP)(lambda: start_qkv(jnp.minimum(nxt, NP - 1)))
        pl.when(nxt == NP + bwslot)(bw_copy.start)
        pl.when(nxt == NP + woslot)(start_wo)

    def transform(j):
        if not opt.get("nopre"):
            pre_qkv(j - 1)
        for m in range(3):
            for t in range(D // 128):
                relayout_tile(j, m, t)

    def relayout_step(j):
        request(j)
        transform(j)

    def relayout_step2(u):
        request(2 * u + 1)
        request(2 * u + 2)
        transform(2 * u + 1)
        transform(2 * u + 2)

    def v_tile(t):
        al = (lambda v, k: v) if isinstance(t, int) else pl.multiple_of
        w = pltpu.bitcast(bw_scr[:, pl.ds(al(2 * D + 128 * t, 128), 128)], bf16)
        wb_scr[2, pl.ds(al(t * 64, 64), 64), :] = pltpu.bitcast(w.T, u32)

    def fold_b_weights(t, last_v):
        al = (lambda v, k: v) if isinstance(t, int) else pl.multiple_of
        lo = al(128 * t, 128)
        r = _iota((4 * GR, 256), 0)
        c = _iota((4 * GR, 256), 1) - 32 * t
        same_head = (c >= 0) & (2 * (r // GR) + r % 2 == jnp.maximum(c, 0) // BDH)
        rf = _iota((4 * GR, BDH), 0) % GR
        et = (_iota((4 * GR, BDH), 1) == 4 * (rf // 8) + (rf % 8) // 2).astype(bf16)
        pm = lax.dot_general(et, wphi_scr[pl.ds(lo, 256), :].astype(bf16), NT, preferred_element_type=f32)
        pm = jnp.where(same_head, pm, 0.0).astype(bf16)
        rows = pl.ds(al(t * 2 * GR, 2 * GR), 2 * GR)
        for m in range(2):
            w = pltpu.bitcast(bw_scr[:, pl.ds(al(m * D + lo, 128), 256)], bf16)
            wb_scr[m, rows, :] = pltpu.bitcast(
                lax.dot_general(pm, w, NT, preferred_element_type=f32).astype(bf16), u32)
        v_tile(t)
        if last_v:
            v_tile(D // 128 - 1)

    def delay(n):
        if n:
            loop(0, n, lambda q: [relayout_tile(NP, m, t) for m in range(3) for t in range(D // 128)])

    delay(opt.get("d_start", 0))
    for m in range(3):
        for p in range(split[0]):
            w_piece(0, m, p, split[0]).wait()
    for j in later:
        start_qkv(j)
    if opt.get("lnmerge", False):
        loop(0, NXP, lambda q: [hpre_chunk(q)] + [relayout_tile(0, m, q) for m in range(3)])
        for m in range(3):
            for t in range(NXP, D // 128):
                relayout_tile(0, m, t)
    else:
        for m in range(3):
            for t in range(D // 128):
                relayout_tile(0, m, t)
    if opt.get("pu2"):
        loop(0, NP // 2, relayout_step2)
    else:
        loop(1, NP + 1, relayout_step)
    if opt.get("prerep"):
        loop(0, opt["prerep"], lambda j: pre_qkv(j % NP))
    if opt.get("relrep"):
        def rr(j):
            j = 1 + j % (NP - 1)
            if not opt.get("nopre"):
                pre_qkv(j - 1)
            for m in range(3):
                for t in range(D // 128):
                    relayout_tile(j, m, t)
        loop(0, opt["relrep"], rr)
    if opt.get("xearly"):
        start_x()
    delay(opt.get("d_mid", 0))
    bw_copy.wait()
    if not opt.get("nofold"):
        fu = opt.get("fold_unroll", 4)
        if fu == 4:
            for t in range(NG // 4):
                fold_b_weights(t, t == 0)
        elif fu == 2:
            loop(0, NG // 8, lambda u: [fold_b_weights(2 * u, True), fold_b_weights(2 * u + 1, False)])
        else:
            loop(0, NG // 4, lambda t: fold_b_weights(t, True))
    delay(opt.get("d_end", 0))
    loop(0, NP, lambda j: w_copy(j, 3).wait())
    if not opt.get("xearly"):
        start_x()
    x_first.wait()

    HB = NG // 2
    ones = jnp.ones((HB, 8, 128), f32)

    def b1_w(m, h):
        r0 = h * 160 if isinstance(h, int) else pl.multiple_of(h * 160, 160)
        return pltpu.bitcast(wb_scr[m, pl.ds(r0, 160), :], bf16)

    def b1_pk(h, xn):
        pk = lax.dot_general(b1_w(1, h), xn, NT, preferred_element_type=f32)
        return _features(pk)

    def b1_v(h, xn, g0=0, g1=HB):
        r0 = h * 160 + g0 * (GR // 2)
        r0 = r0 if isinstance(r0, int) else pl.multiple_of(r0, GR)
        w = pltpu.bitcast(wb_scr[2, pl.ds(r0, (g1 - g0) * (GR // 2)), :], bf16)
        vt = lax.dot_general(w, xn, NT, preferred_element_type=f32)
        return jnp.concatenate([vt.reshape(g1 - g0, GR, 128), ones[g0:g1]], axis=1).astype(bf16)

    VH = HB - opt.get("vtail", 0)

    def b1_lhs(h, xn):
        if VH == 0:
            return lhs_scr[...]
        return jnp.concatenate([b1_v(h, xn, 0, VH), lhs_scr[VH:HB]], axis=0) if VH < HB else b1_v(h, xn)

    def b1_v_next(h, xn):
        lhs_scr[VH:HB] = b1_v(h, xn, VH, HB)

    def b1_pq(b, h, xn):
        pq = lax.dot_general(b1_w(0, h), xn, NT, preferred_element_type=f32)
        phiq_scr[b, pl.ds(pl.multiple_of(h * HB, HB), HB)] = _features(pq)

    def b1_kvt(h, valid, phik, lhs):
        for g in range(HB):
            t = lax.dot_general(lhs[g], phik[g], NT, preferred_element_type=f32)
            if valid is not None:
                t = jnp.where(valid, t, 0.0)
            kvt_scr[h * HB + g] += t

    def store_xnb(slot, val):
        xnb_scr[slot] = val

    def b1_ln(b):
        return _layernorm(x_scr[pl.ds(pl.multiple_of(b * 128, 128), 128), :]).astype(bf16)

    def qkv_cols(h, j, lo, hi):
        w = pltpu.bitcast(wqkv_scr[j, :, lo:hi], bf16)
        return jnp.dot(h, w, preferred_element_type=f32).astype(bf16)

    def a_pass(qkv, keep, fill, pre, post, hooks):
        def oproj(j, o):
            return jnp.dot(o, pltpu.bitcast(wo_scr[j], bf16), preferred_element_type=f32)

        lag = dict(Q=0, S=opt.get("lagS", 1), P=opt.get("lagP", 3), O=opt.get("lagO", 4))
        order = opt.get("order", "QSPO")
        rs, ws, ss, os_ = {}, {}, {}, {}
        acc = None
        for i in range(NP + max(lag.values())):
            for fn in hooks.get(i, ()):
                fn()
            for op in order:
                j = i - lag[op]
                if not (0 <= j < NP):
                    continue
                if op == "Q":
                    rs[j] = qkv(j)
                elif op == "S":
                    ws[j] = pre(j, rs.pop(j))
                    ss[j] = _attn_scores(ws[j][:, 0:PW], ws[j][:, PW:2 * PW])
                elif op == "P":
                    p = _attn_softmax(ss.pop(j), keep, fill)
                    vbd = _blockdiag(ws.pop(j)[:, 2 * PW:3 * PW])
                    o = jnp.dot(p, vbd, preferred_element_type=f32)
                    os_[j] = post(j, o).astype(bf16)
                else:
                    t = oproj(j, os_.pop(j))
                    acc = t if acc is None else acc + t
        for fn in hooks.get(NP + max(lag.values()), ()):
            fn()
        return acc

    def a_layer(l):
        keep_a, fill_a, keep_b, fill_b = _make_masks()
        kvt_scr[...] = jnp.zeros_like(kvt_scr)
        if opt.get("ln0"):
            xnb_scr[0] = b1_ln(0)
        pos = dict(opt.get("pos", dict(K=("a", 0), V=("b", 0), Q=("a", 17), T=("b", 8), L=("b", 4))))
        if VH < HB:
            pos["N"] = opt.get("posN", ("b", 20))

        def step(use_pre, it, mem):
            r0 = pl.multiple_of(it * 64, 64)
            if use_pre:
                pl.when(it == nx0)(x_rest.wait)
                xs = xin_scr[pl.ds(r0, 64), :].astype(f32)
            else:
                xs = x_scr[pl.ds(r0, 64), :]
            xn = _layernorm(xs)
            h_a = jnp.concatenate([mem, xn[0:40]], axis=0).astype(bf16)
            osav = {}

            hb = jnp.maximum(it - 3, 0)
            fb, fh, valid = hb // 2, hb % 2, it >= 3
            st = {}
            fillers = dict(
                K=lambda: st.update(phik=b1_pk(fh, xnb_scr[it % 2])),
                V=lambda: st.update(lhs=b1_lhs(fh, xnb_scr[it % 2])),
                N=lambda: b1_v_next(jnp.maximum(it - 2, 0) % 2, xnb_scr[(it + 1) % 2]),
                Q=lambda: b1_pq(fb, fh, xnb_scr[it % 2]),
                T=lambda: b1_kvt(fh, valid, st["phik"], st["lhs"]),
                L=lambda: store_xnb((it + 1) % 2, b1_ln(jnp.maximum(it - 2, 0) // 2)),
            )
            hooks = {"a": {}, "b": {}}
            if opt.get("fuse", True):
                for name, (ps, slot) in pos.items():
                    hooks[ps].setdefault(slot, []).append(fillers[name])

            def qkv_a(j):
                if use_pre:
                    if opt.get("qfirst", True):
                        r1 = qkv_cols(h_a[0:32], j, 0, PC)
                        r2 = qkv_cols(h_a, j, PC, 3 * PW)
                    else:
                        r2 = qkv_cols(h_a, j, PC, 3 * PW)
                        r1 = qkv_cols(h_a[0:32], j, 0, PC)
                    return r1, r2
                return qkv_cols(h_a, j, 0, 3 * PW)

            def pre_a(j, r):
                if use_pre:
                    sv = pre_scr[j, pl.ds(pl.multiple_of(it * 16, 16), 16), :]
                    sav_scr[j, :, 0:PC] = sv
                    sav_scr[j, :, PC:] = r[1][32:48]
                    return jnp.concatenate([jnp.concatenate([r[0], sv], axis=0), r[1]], axis=1)
                sav_scr[j] = r[32:48]
                return r

            def post_a(j, o):
                osav[j] = o[32:40]
                return o[0:32]

            acc_a = a_pass(qkv_a, keep_a, fill_a, pre_a, post_a, hooks["a"])
            h_b = jnp.concatenate([acc_a[0:8], xn[40:64]], axis=0).astype(bf16)

            def pre_b(j, r):
                return jnp.concatenate([sav_scr[j], r], axis=0)

            def post_b(j, o):
                return jnp.concatenate([osav[j], o[8:48]], axis=0)

            acc_b = a_pass(lambda j: qkv_cols(h_b, j, 0, 3 * PW), keep_b, fill_b, pre_b, post_b, hooks["b"])
            out = jnp.concatenate([acc_a[8:32], acc_b[0:16], acc_b[24:48]], axis=0)
            x_scr[pl.ds(r0, 64), :] = xs + out
            return acc_b[16:24]

        n_var = jnp.where(l == 0, n_pre, 0)
        mem = lax.fori_loop(0, n_var, functools.partial(step, True), mem_ref[...].astype(f32))

        @pl.when(l == 0)
        def _():
            bwo_copy.wait()

        lax.fori_loop(n_var, opt.get("steps", S // 64), functools.partial(step, False), mem)

    def b_layer(l):
        @pl.when(l > 0)
        def _():
            for i in range(NB):
                out_copy(i).wait()

        first = 29 if opt.get("fuse", True) else 0
        if first:
            todo = [(hb // 2, hb % 2) for hb in range(first, 32)]
            if opt.get("left2", True):
                xns = {14: xnb_scr[0], 15: b1_ln(15)}
            else:
                xns = {b: b1_ln(b) for b in sorted({b for b, _ in todo})}
            qlate = opt.get("qlate", 0)
            pend = None
            for n, (b, h) in enumerate(todo):
                phik = b1_pk(h, xns[b])
                if pend is not None:
                    b1_kvt(*pend)
                lhs = b1_lhs(h, xns[b]) if (b, h) == todo[0] else b1_v(h, xns[b])
                if n < len(todo) - qlate:
                    b1_pq(b, h, xns[b])
                pend = (h, None, phik, lhs)
            b1_kvt(*pend)
            late_q = [functools.partial(b1_pq, b, h, xns[b]) for b, h in todo[len(todo) - qlate:]]
        else:
            def p1(hb, c):
                b, h = hb // 2, hb % 2
                xn = b1_ln(b)
                phik = b1_pk(h, xn)
                lhs = b1_v(h, xn)
                b1_pq(b, h, xn)
                b1_kvt(h, None, phik, lhs)
                return c
            lax.fori_loop(0, 32, p1, 0)

        rr = _iota((GR + 8, 2 * GR), 0)
        cc = _iota((GR + 8, 2 * GR), 1)
        m2 = jnp.where(rr < GR, rr // BDH, (rr - GR) // 4) == cc % 2
        for g in range(NG):
            lhs2_scr[g] = jnp.where(m2, kvt_scr[g], 0.0).astype(bf16)
        q_after = opt.get("q_after", 0)
        for fn in late_q[:len(late_q) - q_after]:
            fn()

        lo4 = _iota((8, TB), 0) < 4

        def numden(i):
            outs = []
            for g in range(NG):
                phiq = jnp.concatenate([phiq_scr[2 * i, g], phiq_scr[2 * i + 1, g]], axis=1)
                res = jnp.dot(lhs2_scr[g], phiq, preferred_element_type=f32)
                inv = 1.0 / (res[GR:GR + 8] + 1e-6)
                swp = pltpu.roll(inv, 4, 0)
                i0 = jnp.where(lo4, inv, swp)
                i1 = jnp.where(lo4, swp, inv)
                outs += [res[0:8] * i0, res[8:16] * i0, res[16:24] * inv, res[24:32] * i1, res[32:40] * i1]
            return jnp.concatenate(outs, axis=0).T.astype(bf16)

        def proj(i, o):
            rows = pl.ds(i * TB, TB) if isinstance(i, int) else pl.ds(pl.multiple_of(i * TB, TB), TB)
            xnew = x_scr[rows, :] + jnp.dot(o, pltpu.bitcast(bwo_scr[...], bf16), preferred_element_type=f32)
            x_scr[rows, :] = xnew
            xin_scr[rows, :] = xnew.astype(bf16)
            out_copy(i).start()

        if opt.get("p2pipe", True):
            o_scr[0] = numden(0)
            for fn in late_q[len(late_q) - q_after:]:
                fn()

            def pass2(i, carry):
                o_next = numden(i + 1)
                proj(i, o_scr[i % 2])
                o_scr[(i + 1) % 2] = o_next
                return carry

            lax.fori_loop(0, NB - 1, pass2, 0)
            proj(NB - 1, o_scr[(NB - 1) % 2])
        else:
            lax.fori_loop(0, NB, lambda i, c: (proj(i, numden(i)), c)[1], 0)

    def layer(l, carry):
        if opt.get("A", True):
            a_layer(l)
        else:
            @pl.when(l == 0)
            def _():
                x_rest.wait()
                x_scr[...] = xin_scr[...].astype(f32)
                bwo_copy.wait()
        if opt.get("B", True):
            b_layer(l)
        return carry

    lax.fori_loop(0, 2, layer, 0)
    if not opt.get("B", True):
        for i in range(NB):
            xin_scr[i * TB:(i + 1) * TB, :] = x_scr[i * TB:(i + 1) * TB, :].astype(bf16)
            out_copy(i).start()
    for i in range(NB):
        out_copy(i).wait()


opt = {}
n_pre = S // 64

@jax.jit
def pallas_interleave_layers__memory_aug_recurrent_mem_tr__linear_kernel_hedgehog__prompt_kernel(A_x, A_mem0, A_Wq, A_Wk, A_Wv, A_Wo, A_seg_len, B_x, B_wqkv, B_w_phi, B_wo):
    def tr(w):
        return w.transpose(1, 2, 0).reshape(AH * ADH, D)
    any_spec = pl.BlockSpec(memory_space=pl.ANY)
    out = pl.pallas_call(
        functools.partial(_kernel, opt=opt),
        out_shape=jax.ShapeDtypeStruct((S, D), bf16),
        in_specs=[any_spec] * 10,
        out_specs=any_spec,
        scratch_shapes=[
            pltpu.VMEM((S, D), f32),
            pltpu.VMEM((NP, 16, 3 * PW), bf16),
            pltpu.VMEM((NP + 1, D // 2, 3 * PW), u32),
            pltpu.VMEM((NP, PW // 2, D), u32),
            pltpu.VMEM((3, D // 2, D), u32),
            pltpu.VMEM((D // 2, 3 * D), u32),
            pltpu.VMEM((D // 2, D), u32),
            pltpu.VMEM((S // 128, NG, 2 * GR, 128), bf16),
            pltpu.VMEM((NG, GR + 8, 2 * GR), f32),
            pltpu.VMEM((NG, GR + 8, 2 * GR), bf16),
            pltpu.VMEM((S, D), bf16),
            pltpu.VMEM((3, NP + 1, PW // 2, D), u32),
            pltpu.VMEM((n_pre, 16, D), bf16),
            pltpu.VMEM((n_pre * 16, D), bf16),
            pltpu.VMEM((NP, n_pre * 16, opt.get("PC", 768)), bf16),
            pltpu.VMEM((2, 128, D), bf16),
            pltpu.VMEM((2, TB, D), bf16),
            pltpu.VMEM((D, BDH), f32),
            pltpu.VMEM((M, D), bf16),
            pltpu.VMEM((BDH, BDH, BH), bf16),
            pltpu.VMEM((NG // 2, GR + 8, 128), bf16),
            pltpu.SemaphoreType.DMA((8, NP)),
        ],
        name="fused_layers",
        compiler_params=pltpu.CompilerParams(vmem_limit_bytes=126 * 1024 * 1024),
    )(A_x.reshape(S, D), A_x.reshape(S // 64, 64, D), A_mem0.reshape(M, D), tr(A_Wq), tr(A_Wk), tr(A_Wv), A_Wo.reshape(AH * ADH, D),
      B_wqkv, B_w_phi.transpose(1, 2, 0) if opt.get("wphi3", True) else B_w_phi.reshape(D, BDH), B_wo)
    return out.reshape(1, S, D)
```

```python
import functools
import jax
import jax.numpy as jnp
from jax import lax
from jax.experimental import pallas as pl
from jax.experimental.pallas import tpu as pltpu

S, D = 2048, 640
AH, ADH, M, SEG = 32, 192, 8, 32
NP = AH // 2
PW = 2 * ADH
BH, BDH = 32, 20
NG = BH // 2
GR = 2 * BDH
TB = 256
NB = S // TB
bf16, f32, u32 = jnp.bfloat16, jnp.float32, jnp.uint32
SCALE = ADH ** -0.5
NEG = -1e9
JUNK = -1e30
NT = (((1,), (1,)), ((), ()))
NS = S // 64
PC = 768
NXP = 4
NX0 = 2
WIN = 4
FP = 2
FR = FP * GR
LAG_S, LAG_P, LAG_O = 1, 3, 4


def _layernorm(x):
    m = jnp.mean(x, axis=-1, keepdims=True)
    xc = x - m
    v = jnp.mean(xc * xc, axis=-1, keepdims=True)
    return xc * lax.rsqrt(v + 1e-5)


def _iota(shape, dim):
    return lax.broadcasted_iota(jnp.int32, shape, dim)


def _make_masks():
    r = _iota((48, 96), 0)
    c = _iota((48, 96), 1)
    c = jnp.where(c >= 48, c - 48, c)
    valid_a = c < 40
    keep_a = ((r < 8) | (r >= c)) & valid_a
    fill_a = jnp.where(valid_a, NEG, JUNK).astype(f32)
    lr = jnp.where(r < 16, r, jnp.where(r < 24, r - 16, r - 8))
    lc = jnp.where(c < 16, c, jnp.where(c < 24, c - 16, c - 8))
    valid_b = c >= 8
    keep_b = ((lr < 8) | (lr >= lc)) & valid_b
    fill_b = jnp.where(valid_b, NEG, JUNK).astype(f32)
    return keep_a, fill_a, keep_b, fill_b


def _blockdiag(k):
    ku = pltpu.bitcast(k, u32)
    lo = _iota(ku.shape, 1) < ADH
    z = jnp.zeros_like(ku)
    return pltpu.bitcast(jnp.concatenate([jnp.where(lo, ku, z), jnp.where(lo, z, ku)], axis=0), bf16)


def _attn_scores(q, k):
    return lax.dot_general(q, _blockdiag(k), NT, preferred_element_type=f32)


def _attn_softmax(s, keep, fill):
    s = jnp.where(keep, s * SCALE, fill)
    h0 = _iota((48, 96), 1) < 48
    m0 = jnp.max(jnp.where(h0, s, -jnp.inf), axis=-1, keepdims=True)
    m1 = jnp.max(jnp.where(h0, -jnp.inf, s), axis=-1, keepdims=True)
    e = jnp.exp(s - jnp.where(h0, m0, m1))
    l0 = jnp.sum(jnp.where(h0, e, 0.0), axis=-1, keepdims=True)
    l1 = jnp.sum(jnp.where(h0, 0.0, e), axis=-1, keepdims=True)
    return (e * jnp.where(h0, 1.0 / l0, 1.0 / l1)).astype(bf16)


def _pair_reduce(op, a):
    a = op(a, pltpu.roll(a, 2, 1))
    return op(a, pltpu.roll(a, 4, 1))


def _features(p):
    t = p.shape[-1]
    ng = p.shape[0] // GR
    p4 = p.reshape(ng, 5, 8, t)
    mx = _pair_reduce(jnp.maximum, jnp.max(p4, axis=1))[:, None]
    mn = _pair_reduce(jnp.minimum, jnp.min(p4, axis=1))[:, None]
    ep = jnp.exp(p4 - mx)
    en = jnp.exp(mn - p4)
    pos = ep * (1.0 / _pair_reduce(jnp.add, jnp.sum(ep, axis=1)))[:, None]
    neg = en * (1.0 / _pair_reduce(jnp.add, jnp.sum(en, axis=1)))[:, None]
    return jnp.concatenate([pos, neg], axis=1).reshape(ng, 2 * GR, t).astype(bf16)


def _kernel(x_hbm, x3_hbm, mem_hbm, wq_hbm, wk_hbm, wv_hbm, wo_hbm, bw_hbm, wphi_hbm, bwo_hbm, o_hbm,
            x_scr, sav_scr, wqkv_scr, wo_scr, wb_scr, bw_scr, bwo_scr, phiq_scr, kvt_scr, lhs2_scr,
            xin_scr, stage_scr, xpre_scr, hpre_scr, pre_scr, xnb_scr, o_scr, wphi_scr, mem_ref, wphi_ref, sems):
    w_hbm = tuple(w.bitcast(u32) for w in (wq_hbm, wk_hbm, wv_hbm, wo_hbm))

    def w_copy(j, m):
        dst = wo_scr.at[j] if m == 3 else stage_scr.at[m, j]
        r0 = j * (PW // 2) if isinstance(j, int) else pl.multiple_of(j * (PW // 2), PW // 2)
        return pltpu.make_async_copy(w_hbm[m].at[pl.ds(r0, PW // 2), :], dst, sems.at[m, j])

    def out_copy(i):
        return pltpu.make_async_copy(xin_scr.at[pl.ds(i * TB, TB), :], o_hbm.at[pl.ds(i * TB, TB), :],
                                     sems.at[5, i])

    def xpre_copy(q):
        steps = pl.ds(q * (NS // NXP), NS // NXP)
        return pltpu.make_async_copy(x3_hbm.at[steps, pl.ds(24, 16), :], xpre_scr.at[steps], sems.at[6, q])

    x_first = pltpu.make_async_copy(x_hbm.at[pl.ds(0, NX0 * 64), :], xin_scr.at[pl.ds(0, NX0 * 64), :], sems.at[7, 0])
    x_rest = pltpu.make_async_copy(x_hbm.at[pl.ds(NX0 * 64, S - NX0 * 64), :],
                                   xin_scr.at[pl.ds(NX0 * 64, S - NX0 * 64), :], sems.at[7, 1])
    bw_copy = pltpu.make_async_copy(bw_hbm.bitcast(u32), bw_scr, sems.at[4, 1])
    bwo_copy = pltpu.make_async_copy(bwo_hbm.bitcast(u32), bwo_scr, sems.at[4, 2])
    mem_copy = pltpu.make_async_copy(mem_hbm, mem_ref, sems.at[4, 4])
    wphi_copy = pltpu.make_async_copy(wphi_hbm, wphi_ref, sems.at[4, 5])

    def loop(lo, hi, fn):
        lax.fori_loop(lo, hi, lambda i, c: (fn(i), c)[1], 0)

    def start_qkv(j):
        w_copy(j, 0).start()
        w_copy(j, 1).start()
        w_copy(j - 1, 2).start()

    for q in range(NXP):
        xpre_copy(q).start()
    w_copy(0, 0).start()
    w_copy(0, 1).start()
    loop(1, WIN, start_qkv)
    x_first.start()
    mem_copy.start()
    wphi_copy.start()

    x_scr[0:128, :] = jnp.zeros((128, D), f32)
    xnb_scr[...] = jnp.zeros(xnb_scr.shape, bf16)

    def hpre_chunk(q):
        xpre_copy(q).wait()
        xq = xpre_scr[pl.ds(q * (NS // NXP), NS // NXP)].reshape(128, D).astype(f32)
        hpre_scr[pl.ds(pl.multiple_of(q * 128, 128), 128), :] = _layernorm(xq).astype(bf16)

    loop(0, NXP, hpre_chunk)

    def relayout(j, m):
        for t in range(D // 128):
            blk = pltpu.bitcast(stage_scr[m, j, :, t * 128:(t + 1) * 128], bf16)
            wqkv_scr[j, t * 64:(t + 1) * 64, m * PW:(m + 1) * PW] = pltpu.bitcast(blk.T, u32)

    def weight_step(j):
        @pl.when(j < NP)
        def _():
            w_copy(j, 0).wait()
            w_copy(j, 1).wait()

        w_copy(j - 1, 2).wait()
        nxt = j + WIN - 1
        pl.when(nxt < NP)(lambda: start_qkv(jnp.minimum(nxt, NP - 1)))
        pl.when(nxt == NP)(lambda: w_copy(NP - 1, 2).start())
        pl.when(nxt == NP)(bw_copy.start)
        w_copy(j - 1, 3).start()
        pre_scr[j - 1] = jnp.dot(hpre_scr[...], pltpu.bitcast(wqkv_scr[j - 1, :, 0:PC], bf16),
                                 preferred_element_type=f32).astype(bf16)
        relayout(j, 0)
        relayout(j, 1)
        relayout(j - 1, 2)

    def fold_window(t):
        return 128 * (FR * t // 128), 128 * -(-FR * (t + 1) // 128)

    def fold_matrix(t):
        lo, hi = fold_window(t)
        r = _iota((FR, hi - lo), 0)
        c = _iota((FR, hi - lo), 1) + (lo - FR * t)
        same_head = (c >= 0) & (2 * (r // GR) + r % 2 == jnp.maximum(c, 0) // BDH)
        rf = _iota((FR, BDH), 0) % GR
        et = (_iota((FR, BDH), 1) == 4 * (rf // 8) + (rf % 8) // 2).astype(bf16)
        pm = lax.dot_general(et, wphi_scr[lo:hi, :].astype(bf16), NT, preferred_element_type=f32)
        return jnp.where(same_head, pm, 0.0).astype(bf16)

    w_copy(0, 0).wait()
    w_copy(0, 1).wait()
    relayout(0, 0)
    relayout(0, 1)
    loop(1, NP + 1, weight_step)

    bw_copy.wait()
    mem_copy.wait()
    wphi_copy.wait()
    for e in range(BDH):
        wphi_scr[pl.ds(e, BH, stride=BDH), :] = wphi_ref[e].astype(f32).T
    pms = [fold_matrix(t) for t in range(NG // FP)]
    for t in range(NG // FP):
        lo, hi = fold_window(t)
        for m in range(2):
            w = pltpu.bitcast(bw_scr[:, m * D + lo:m * D + hi], bf16)
            wb_scr[m, t * FR // 2:(t + 1) * FR // 2, :] = pltpu.bitcast(
                lax.dot_general(pms[t], w, NT, preferred_element_type=f32).astype(bf16), u32)
    for t in range(D // 128):
        w = pltpu.bitcast(bw_scr[:, 2 * D + 128 * t:2 * D + 128 * (t + 1)], bf16)
        wb_scr[2, t * 64:(t + 1) * 64, :] = pltpu.bitcast(w.T, u32)

    loop(0, NP, lambda j: w_copy(j, 3).wait())
    x_rest.start()
    bwo_copy.start()
    x_first.wait()

    HB = NG // 2
    ones = jnp.ones((HB, 8, 128), f32)

    def b1_w(m, h):
        r0 = h * 160 if isinstance(h, int) else pl.multiple_of(h * 160, 160)
        return pltpu.bitcast(wb_scr[m, pl.ds(r0, 160), :], bf16)

    def b1_pk(h, xn):
        pk = lax.dot_general(b1_w(1, h), xn, NT, preferred_element_type=f32)
        return _features(pk)

    def b1_v(h, xn):
        vt = lax.dot_general(b1_w(2, h), xn, NT, preferred_element_type=f32)
        return jnp.concatenate([vt.reshape(HB, GR, 128), ones], axis=1).astype(bf16)

    def b1_pq(b, h, xn):
        pq = lax.dot_general(b1_w(0, h), xn, NT, preferred_element_type=f32)
        phiq_scr[b, pl.ds(pl.multiple_of(h * HB, HB), HB)] = _features(pq)

    def b1_kvt(h, valid, phik, lhs):
        for g in range(HB):
            t = lax.dot_general(lhs[g], phik[g], NT, preferred_element_type=f32)
            if valid is not None:
                t = jnp.where(valid, t, 0.0)
            kvt_scr[h * HB + g] += t

    def b1_ln(b):
        return _layernorm(x_scr[pl.ds(pl.multiple_of(b * 128, 128), 128), :]).astype(bf16)

    def qkv_cols(h, j, lo, hi):
        w = pltpu.bitcast(wqkv_scr[j, :, lo:hi], bf16)
        return jnp.dot(h, w, preferred_element_type=f32).astype(bf16)

    def a_pass(qkv, keep, fill, pre, post, hooks):
        def oproj(j, o):
            return jnp.dot(o, pltpu.bitcast(wo_scr[j], bf16), preferred_element_type=f32)

        rs, ws, ss, os_ = {}, {}, {}, {}
        acc = None
        for i in range(NP + LAG_O + 1):
            for fn in hooks.get(i, ()):
                fn()
            if i < NP:
                rs[i] = qkv(i)
            j = i - LAG_S
            if 0 <= j < NP:
                ws[j] = pre(j, rs.pop(j))
                ss[j] = _attn_scores(ws[j][:, 0:PW], ws[j][:, PW:2 * PW])
            j = i - LAG_P
            if 0 <= j < NP:
                p = _attn_softmax(ss.pop(j), keep, fill)
                vbd = _blockdiag(ws.pop(j)[:, 2 * PW:3 * PW])
                o = jnp.dot(p, vbd, preferred_element_type=f32)
                os_[j] = post(j, o).astype(bf16)
            j = i - LAG_O
            if 0 <= j < NP:
                t = oproj(j, os_.pop(j))
                acc = t if acc is None else acc + t
        return acc

    def a_layer(l):
        keep_a, fill_a, keep_b, fill_b = _make_masks()
        kvt_scr[...] = jnp.zeros_like(kvt_scr)

        def step(use_pre, it, mem):
            r0 = pl.multiple_of(it * 64, 64)
            if use_pre:
                pl.when(it == NX0)(x_rest.wait)
                xs = xin_scr[pl.ds(r0, 64), :].astype(f32)
            else:
                xs = x_scr[pl.ds(r0, 64), :]
            xn = _layernorm(xs)
            h_a = jnp.concatenate([mem, xn[0:40]], axis=0).astype(bf16)
            osav = {}

            hq = jnp.maximum(it - 3, 0)
            hk = jnp.maximum(it - 2, 0)
            st = {}

            def fill_q():
                b1_pq(hq // 2, hq % 2, xnb_scr[(it + 1) % 2])

            def fill_ln():
                xnb_scr[it % 2] = b1_ln(hk // 2)

            def fill_k():
                st["phik"] = b1_pk(hk % 2, xnb_scr[it % 2])

            def fill_v():
                st["lhs"] = b1_v(hk % 2, xnb_scr[it % 2])

            def fill_t():
                b1_kvt(hk % 2, it >= 2, st["phik"], st["lhs"])

            def qkv_a(j):
                if use_pre:
                    return qkv_cols(h_a[0:32], j, 0, PC), qkv_cols(h_a, j, PC, 3 * PW)
                return qkv_cols(h_a, j, 0, 3 * PW)

            def pre_a(j, r):
                if use_pre:
                    sv = pre_scr[j, pl.ds(pl.multiple_of(it * 16, 16), 16), :]
                    sav_scr[j, :, 0:PC] = sv
                    sav_scr[j, :, PC:] = r[1][32:48]
                    return jnp.concatenate([jnp.concatenate([r[0], sv], axis=0), r[1]], axis=1)
                sav_scr[j] = r[32:48]
                return r

            def post_a(j, o):
                osav[j] = o[32:40]
                return o[0:32]

            acc_a = a_pass(qkv_a, keep_a, fill_a, pre_a, post_a,
                           {0: [fill_q], 10: [fill_ln], NP + 1: [fill_k]})
            h_b = jnp.concatenate([acc_a[0:8], xn[40:64]], axis=0).astype(bf16)

            def pre_b(j, r):
                return jnp.concatenate([sav_scr[j], r], axis=0)

            def post_b(j, o):
                return jnp.concatenate([osav[j], o[8:48]], axis=0)

            acc_b = a_pass(lambda j: qkv_cols(h_b, j, 0, 3 * PW), keep_b, fill_b, pre_b, post_b,
                           {0: [fill_v], NP + LAG_O: [fill_t]})
            out = jnp.concatenate([acc_a[8:32], acc_b[0:16], acc_b[24:48]], axis=0)
            x_scr[pl.ds(r0, 64), :] = xs + out
            return acc_b[16:24]

        n_pre = jnp.where(l == 0, NS, 0)
        mem = lax.fori_loop(0, n_pre, functools.partial(step, True), mem_ref[...].astype(f32))
        pl.when(l == 0)(bwo_copy.wait)
        lax.fori_loop(n_pre, NS, functools.partial(step, False), mem)

    def b_layer(l):
        @pl.when(l > 0)
        def _():
            for i in range(NB):
                out_copy(i).wait()

        last = S // 128 - 1
        xl = b1_ln(last)
        b1_pq(last - 1, 1, xnb_scr[1])
        pend = None
        for h in range(2):
            phik = b1_pk(h, xl)
            if pend is not None:
                b1_kvt(*pend)
            lhs = b1_v(h, xl)
            b1_pq(last, h, xl)
            pend = (h, None, phik, lhs)
        b1_kvt(*pend)

        rr = _iota((GR + 8, 2 * GR), 0)
        cc = _iota((GR + 8, 2 * GR), 1)
        m2 = jnp.where(rr < GR, rr // BDH, (rr - GR) // 4) == cc % 2
        for g in range(NG):
            lhs2_scr[g] = jnp.where(m2, kvt_scr[g], 0.0).astype(bf16)

        lo4 = _iota((8, TB), 0) < 4

        def numden(i):
            outs = []
            for g in range(NG):
                phiq = jnp.concatenate([phiq_scr[2 * i, g], phiq_scr[2 * i + 1, g]], axis=1)
                res = jnp.dot(lhs2_scr[g], phiq, preferred_element_type=f32)
                inv = 1.0 / (res[GR:GR + 8] + 1e-6)
                swp = pltpu.roll(inv, 4, 0)
                i0 = jnp.where(lo4, inv, swp)
                i1 = jnp.where(lo4, swp, inv)
                outs += [res[0:8] * i0, res[8:16] * i0, res[16:24] * inv, res[24:32] * i1, res[32:40] * i1]
            return jnp.concatenate(outs, axis=0).T.astype(bf16)

        def proj(i, o):
            rows = pl.ds(i * TB, TB) if isinstance(i, int) else pl.ds(pl.multiple_of(i * TB, TB), TB)
            xnew = x_scr[rows, :] + jnp.dot(o, pltpu.bitcast(bwo_scr[...], bf16), preferred_element_type=f32)
            x_scr[rows, :] = xnew
            xin_scr[rows, :] = xnew.astype(bf16)
            out_copy(i).start()

        o_scr[...] = numden(0)

        def pass2(u, carry):
            o1 = numden(2 * u + 1)
            proj(2 * u, o_scr[...])
            o2 = numden(2 * u + 2)
            proj(2 * u + 1, o1)
            o_scr[...] = o2
            return carry

        lax.fori_loop(0, NB // 2 - 1, pass2, 0)
        o1 = numden(NB - 1)
        proj(NB - 2, o_scr[...])
        proj(NB - 1, o1)

    def layer(l, carry):
        a_layer(l)
        b_layer(l)
        return carry

    lax.fori_loop(0, 2, layer, 0)
    for i in range(NB):
        out_copy(i).wait()


@jax.jit
def pallas_interleave_layers__memory_aug_recurrent_mem_tr__linear_kernel_hedgehog__prompt_kernel(A_x, A_mem0, A_Wq, A_Wk, A_Wv, A_Wo, A_seg_len, B_x, B_wqkv, B_w_phi, B_wo):
    def tr(w):
        return w.transpose(1, 2, 0).reshape(AH * ADH, D)
    out = pl.pallas_call(
        _kernel,
        out_shape=jax.ShapeDtypeStruct((S, D), bf16),
        in_specs=[pl.BlockSpec(memory_space=pl.ANY)] * 10,
        out_specs=pl.BlockSpec(memory_space=pl.ANY),
        scratch_shapes=[
            pltpu.VMEM((S, D), f32),
            pltpu.VMEM((NP, 16, 3 * PW), bf16),
            pltpu.VMEM((NP + 1, D // 2, 3 * PW), u32),
            pltpu.VMEM((NP, PW // 2, D), u32),
            pltpu.VMEM((3, D // 2, D), u32),
            pltpu.VMEM((D // 2, 3 * D), u32),
            pltpu.VMEM((D // 2, D), u32),
            pltpu.VMEM((S // 128, NG, 2 * GR, 128), bf16),
            pltpu.VMEM((NG, GR + 8, 2 * GR), f32),
            pltpu.VMEM((NG, GR + 8, 2 * GR), bf16),
            pltpu.VMEM((S, D), bf16),
            pltpu.VMEM((3, NP + 1, PW // 2, D), u32),
            pltpu.VMEM((NS, 16, D), bf16),
            pltpu.VMEM((NS * 16, D), bf16),
            pltpu.VMEM((NP, NS * 16, PC), bf16),
            pltpu.VMEM((2, 128, D), bf16),
            pltpu.VMEM((TB, D), bf16),
            pltpu.VMEM((D, BDH), f32),
            pltpu.VMEM((M, D), bf16),
            pltpu.VMEM((BDH, BDH, BH), bf16),
            pltpu.SemaphoreType.DMA((8, NP)),
        ],
        name="fused_layers",
        compiler_params=pltpu.CompilerParams(vmem_limit_bytes=126 * 1024 * 1024),
    )(A_x.reshape(S, D), A_x.reshape(NS, 64, D), A_mem0.reshape(M, D), tr(A_Wq), tr(A_Wk), tr(A_Wv),
      A_Wo.reshape(AH * ADH, D), B_wqkv, B_w_phi.transpose(1, 2, 0), B_wo)
    return out.reshape(1, S, D)
```

```python
import functools
import jax
import jax.numpy as jnp
from jax import lax
from jax.experimental import pallas as pl
from jax.experimental.pallas import tpu as pltpu

S, D = 2048, 640
AH, ADH, M, SEG = 32, 192, 8, 32
NP = AH // 2
PW = 2 * ADH
BH, BDH = 32, 20
NG = BH // 2
GR = 2 * BDH
TB = 256
NB = S // TB
bf16, f32, u32 = jnp.bfloat16, jnp.float32, jnp.uint32
SCALE = ADH ** -0.5
NEG = -1e9
JUNK = -1e30
NT = (((1,), (1,)), ((), ()))
NS = S // 64
PC = 768
NXP = 4
NX0 = 2
WIN = 4
FP = 2
FR = FP * GR
SEM_WO, SEM_OUT, SEM_XPRE = 3 * WIN, 3 * WIN + 1, 3 * WIN + 2
SEM_MISC = SEM_XPRE + NXP
LAG_S, LAG_P, LAG_O = 1, 3, 4


def _layernorm(x):
    m = jnp.mean(x, axis=-1, keepdims=True)
    xc = x - m
    v = jnp.mean(xc * xc, axis=-1, keepdims=True)
    return xc * lax.rsqrt(v + 1e-5)


def _iota(shape, dim):
    return lax.broadcasted_iota(jnp.int32, shape, dim)


def _make_masks():
    r = _iota((48, 96), 0)
    c = _iota((48, 96), 1)
    c = jnp.where(c >= 48, c - 48, c)
    valid_a = c < 40
    keep_a = ((r < 8) | (r >= c)) & valid_a
    fill_a = jnp.where(valid_a, NEG, JUNK).astype(f32)
    lr = jnp.where(r < 16, r, jnp.where(r < 24, r - 16, r - 8))
    lc = jnp.where(c < 16, c, jnp.where(c < 24, c - 16, c - 8))
    valid_b = c >= 8
    keep_b = ((lr < 8) | (lr >= lc)) & valid_b
    fill_b = jnp.where(valid_b, NEG, JUNK).astype(f32)
    return keep_a, fill_a, keep_b, fill_b


def _blockdiag(k):
    ku = pltpu.bitcast(k, u32)
    lo = _iota(ku.shape, 1) < ADH
    z = jnp.zeros_like(ku)
    return pltpu.bitcast(jnp.concatenate([jnp.where(lo, ku, z), jnp.where(lo, z, ku)], axis=0), bf16)


def _attn_scores(q, k):
    return lax.dot_general(q, _blockdiag(k), NT, preferred_element_type=f32)


def _attn_softmax(s, keep, fill):
    s = jnp.where(keep, s * SCALE, fill)
    h0 = _iota((48, 96), 1) < 48
    m0 = jnp.max(jnp.where(h0, s, -jnp.inf), axis=-1, keepdims=True)
    m1 = jnp.max(jnp.where(h0, -jnp.inf, s), axis=-1, keepdims=True)
    e = jnp.exp(s - jnp.where(h0, m0, m1))
    l0 = jnp.sum(jnp.where(h0, e, 0.0), axis=-1, keepdims=True)
    l1 = jnp.sum(jnp.where(h0, 0.0, e), axis=-1, keepdims=True)
    return (e * jnp.where(h0, 1.0 / l0, 1.0 / l1)).astype(bf16)


def _pair_reduce(op, a):
    a = op(a, pltpu.roll(a, 2, 1))
    return op(a, pltpu.roll(a, 4, 1))


def _features(p):
    t = p.shape[-1]
    ng = p.shape[0] // GR
    p4 = p.reshape(ng, 5, 8, t)
    mx = _pair_reduce(jnp.maximum, jnp.max(p4, axis=1))[:, None]
    mn = _pair_reduce(jnp.minimum, jnp.min(p4, axis=1))[:, None]
    ep = jnp.exp(p4 - mx)
    en = jnp.exp(mn - p4)
    pos = ep * (1.0 / _pair_reduce(jnp.add, jnp.sum(ep, axis=1)))[:, None]
    neg = en * (1.0 / _pair_reduce(jnp.add, jnp.sum(en, axis=1)))[:, None]
    return jnp.concatenate([pos, neg], axis=1).reshape(ng, 2 * GR, t).astype(bf16)


def _kernel(x_hbm, x3_hbm, mem_hbm, wq_hbm, wk_hbm, wv_hbm, wo_hbm, bw_hbm, wphi_hbm, bwo_hbm, o_hbm,
            x_scr, sav_scr, wqkv_scr, wo_scr, wb_scr, bw_scr, bwo_scr, phiq_scr, kvt_scr, lhs2_scr,
            xin_scr, stage_scr, xpre_scr, hpre_scr, pre_scr, xnb_scr, o_scr, wphi_scr, mem_ref, wphi_ref, pm_scr, sems):
    w_hbm = tuple(w.bitcast(u32) for w in (wq_hbm, wk_hbm, wv_hbm, wo_hbm))

    def w_copy(j, m):
        dst = wo_scr.at[j] if m == 3 else stage_scr.at[m, j]
        r0 = j * (PW // 2) if isinstance(j, int) else pl.multiple_of(j * (PW // 2), PW // 2)
        sem = sems.at[SEM_WO] if m == 3 else sems.at[m * WIN + j % WIN]
        return pltpu.make_async_copy(w_hbm[m].at[pl.ds(r0, PW // 2), :], dst, sem)

    def out_copy(i):
        return pltpu.make_async_copy(xin_scr.at[pl.ds(i * TB, TB), :], o_hbm.at[pl.ds(i * TB, TB), :],
                                     sems.at[SEM_OUT])

    def xpre_copy(q):
        steps = pl.ds(q * (NS // NXP), NS // NXP)
        return pltpu.make_async_copy(x3_hbm.at[steps, pl.ds(24, 16), :], xpre_scr.at[steps], sems.at[SEM_XPRE + q])

    x_first = pltpu.make_async_copy(x_hbm.at[pl.ds(0, NX0 * 64), :], xin_scr.at[pl.ds(0, NX0 * 64), :], sems.at[SEM_MISC])
    x_rest = pltpu.make_async_copy(x_hbm.at[pl.ds(NX0 * 64, S - NX0 * 64), :],
                                   xin_scr.at[pl.ds(NX0 * 64, S - NX0 * 64), :], sems.at[SEM_MISC + 1])
    bw_copy = pltpu.make_async_copy(bw_hbm.bitcast(u32), bw_scr, sems.at[SEM_MISC + 2])
    bwo_copy = pltpu.make_async_copy(bwo_hbm.bitcast(u32), bwo_scr, sems.at[SEM_MISC + 3])
    mem_copy = pltpu.make_async_copy(mem_hbm, mem_ref, sems.at[SEM_MISC + 4])
    wphi_copy = pltpu.make_async_copy(wphi_hbm, wphi_ref, sems.at[SEM_MISC + 5])

    def loop(lo, hi, fn):
        lax.fori_loop(lo, hi, lambda i, c: (fn(i), c)[1], 0)

    def start_qkv(j):
        w_copy(j, 0).start()
        w_copy(j, 1).start()
        w_copy(j - 1, 2).start()

    wphi_copy.start()
    for q in range(NXP):
        xpre_copy(q).start()
    w_copy(0, 0).start()
    w_copy(0, 1).start()
    loop(1, WIN, start_qkv)

    x_scr[0:128, :] = jnp.zeros((128, D), f32)
    xnb_scr[...] = jnp.zeros(xnb_scr.shape, bf16)

    def hpre_chunk(q):
        xpre_copy(q).wait()
        xq = xpre_scr[pl.ds(q * (NS // NXP), NS // NXP)].reshape(128, D).astype(f32)
        hpre_scr[pl.ds(pl.multiple_of(q * 128, 128), 128), :] = _layernorm(xq).astype(bf16)

    loop(0, NXP, hpre_chunk)

    def relayout(j, m):
        for t in range(D // 128):
            blk = pltpu.bitcast(stage_scr[m, j, :, t * 128:(t + 1) * 128], bf16)
            wqkv_scr[j, t * 64:(t + 1) * 64, m * PW:(m + 1) * PW] = pltpu.bitcast(blk.T, u32)

    def weight_step(j):
        @pl.when(j < NP)
        def _():
            w_copy(j, 0).wait()
            w_copy(j, 1).wait()

        w_copy(j - 1, 2).wait()
        nxt = j + WIN - 1
        pl.when(nxt < NP)(lambda: start_qkv(jnp.minimum(nxt, NP - 1)))

        @pl.when(nxt == NP)
        def _():
            w_copy(NP - 1, 2).start()
            bw_copy.start()
            x_first.start()
            mem_copy.start()

        w_copy(j - 1, 3).start()
        pre_scr[j - 1] = jnp.dot(hpre_scr[...], pltpu.bitcast(wqkv_scr[j - 1, :, 0:PC], bf16),
                                 preferred_element_type=f32).astype(bf16)
        relayout(j, 0)
        relayout(j, 1)
        relayout(j - 1, 2)

    def fold_window(t):
        return 128 * (FR * t // 128), 128 * -(-FR * (t + 1) // 128)

    def fold_matrix(t):
        lo, hi = fold_window(t)
        r = _iota((FR, hi - lo), 0)
        c = _iota((FR, hi - lo), 1) + (lo - FR * t)
        same_head = (c >= 0) & (2 * (r // GR) + r % 2 == jnp.maximum(c, 0) // BDH)
        rf = _iota((FR, BDH), 0) % GR
        et = (_iota((FR, BDH), 1) == 4 * (rf // 8) + (rf % 8) // 2).astype(bf16)
        pm = lax.dot_general(et, wphi_scr[lo:hi, :].astype(bf16), NT, preferred_element_type=f32)
        return jnp.where(same_head, pm, 0.0).astype(bf16)

    wphi_copy.wait()
    for e in range(BDH):
        wphi_scr[pl.ds(e, BH, stride=BDH), :] = wphi_ref[e].astype(f32).T
    for t in range(NG // FP):
        lo, hi = fold_window(t)
        pm_scr[t, :, 0:hi - lo] = fold_matrix(t)

    w_copy(0, 0).wait()
    w_copy(0, 1).wait()
    relayout(0, 0)
    relayout(0, 1)
    loop(1, NP + 1, weight_step)

    bw_copy.wait()
    mem_copy.wait()
    for t in range(NG // FP):
        lo, hi = fold_window(t)
        for m in range(2):
            w = pltpu.bitcast(bw_scr[:, m * D + lo:m * D + hi], bf16)
            wb_scr[m, t * FR // 2:(t + 1) * FR // 2, :] = pltpu.bitcast(
                lax.dot_general(pm_scr[t, :, 0:hi - lo], w, NT, preferred_element_type=f32).astype(bf16), u32)
    for t in range(D // 128):
        w = pltpu.bitcast(bw_scr[:, 2 * D + 128 * t:2 * D + 128 * (t + 1)], bf16)
        wb_scr[2, t * 64:(t + 1) * 64, :] = pltpu.bitcast(w.T, u32)

    loop(0, NP, lambda j: w_copy(j, 3).wait())
    x_rest.start()
    bwo_copy.start()
    x_first.wait()

    HB = NG // 2
    ones = jnp.ones((HB, 8, 128), f32)

    def b1_w(m, h):
        r0 = h * 160 if isinstance(h, int) else pl.multiple_of(h * 160, 160)
        return pltpu.bitcast(wb_scr[m, pl.ds(r0, 160), :], bf16)

    def b1_pk(h, xn):
        pk = lax.dot_general(b1_w(1, h), xn, NT, preferred_element_type=f32)
        return _features(pk)

    def b1_v(h, xn):
        vt = lax.dot_general(b1_w(2, h), xn, NT, preferred_element_type=f32)
        return jnp.concatenate([vt.reshape(HB, GR, 128), ones], axis=1).astype(bf16)

    def b1_pq(b, h, xn):
        pq = lax.dot_general(b1_w(0, h), xn, NT, preferred_element_type=f32)
        phiq_scr[b, pl.ds(pl.multiple_of(h * HB, HB), HB)] = _features(pq)

    def b1_kvt(h, valid, phik, lhs):
        for g in range(HB):
            t = lax.dot_general(lhs[g], phik[g], NT, preferred_element_type=f32)
            if valid is not None:
                t = jnp.where(valid, t, 0.0)
            kvt_scr[h * HB + g] += t

    def b1_ln(b):
        return _layernorm(x_scr[pl.ds(pl.multiple_of(b * 128, 128), 128), :]).astype(bf16)

    def qkv_cols(h, j, lo, hi):
        w = pltpu.bitcast(wqkv_scr[j, :, lo:hi], bf16)
        return jnp.dot(h, w, preferred_element_type=f32).astype(bf16)

    def a_pass(qkv, keep, fill, pre, post, hooks):
        def oproj(j, o):
            return jnp.dot(o, pltpu.bitcast(wo_scr[j], bf16), preferred_element_type=f32)

        rs, ws, ss, os_ = {}, {}, {}, {}
        acc = None
        for i in range(NP + LAG_O + 1):
            for fn in hooks.get(i, ()):
                fn()
            if i < NP:
                rs[i] = qkv(i)
            j = i - LAG_S
            if 0 <= j < NP:
                ws[j] = pre(j, rs.pop(j))
                ss[j] = _attn_scores(ws[j][:, 0:PW], ws[j][:, PW:2 * PW])
            j = i - LAG_P
            if 0 <= j < NP:
                p = _attn_softmax(ss.pop(j), keep, fill)
                vbd = _blockdiag(ws.pop(j)[:, 2 * PW:3 * PW])
                o = jnp.dot(p, vbd, preferred_element_type=f32)
                os_[j] = post(j, o).astype(bf16)
            j = i - LAG_O
            if 0 <= j < NP:
                t = oproj(j, os_.pop(j))
                acc = t if acc is None else acc + t
        return acc

    def a_layer(l):
        keep_a, fill_a, keep_b, fill_b = _make_masks()
        kvt_scr[...] = jnp.zeros_like(kvt_scr)

        def step(use_pre, it, mem):
            r0 = pl.multiple_of(it * 64, 64)
            if use_pre:
                pl.when(it == NX0)(x_rest.wait)
                xs = xin_scr[pl.ds(r0, 64), :].astype(f32)
            else:
                xs = x_scr[pl.ds(r0, 64), :]
            xn = _layernorm(xs)
            h_a = jnp.concatenate([mem, xn[0:40]], axis=0).astype(bf16)
            osav = {}

            hq = jnp.maximum(it - 3, 0)
            hk = jnp.maximum(it - 2, 0)
            st = {}

            def fill_q():
                b1_pq(hq // 2, hq % 2, xnb_scr[(it + 1) % 2])

            def fill_ln():
                xnb_scr[it % 2] = b1_ln(hk // 2)

            def fill_k():
                st["phik"] = b1_pk(hk % 2, xnb_scr[it % 2])

            def fill_v():
                st["lhs"] = b1_v(hk % 2, xnb_scr[it % 2])

            def fill_t():
                b1_kvt(hk % 2, it >= 2, st["phik"], st["lhs"])

            def qkv_a(j):
                if use_pre:
                    return qkv_cols(h_a[0:32], j, 0, PC), qkv_cols(h_a, j, PC, 3 * PW)
                return qkv_cols(h_a, j, 0, 3 * PW)

            def pre_a(j, r):
                if use_pre:
                    sv = pre_scr[j, pl.ds(pl.multiple_of(it * 16, 16), 16), :]
                    sav_scr[j, :, 0:PC] = sv
                    sav_scr[j, :, PC:] = r[1][32:48]
                    return jnp.concatenate([jnp.concatenate([r[0], sv], axis=0), r[1]], axis=1)
                sav_scr[j] = r[32:48]
                return r

            def post_a(j, o):
                osav[j] = o[32:40]
                return o[0:32]

            acc_a = a_pass(qkv_a, keep_a, fill_a, pre_a, post_a,
                           {0: [fill_q], 10: [fill_ln], NP + 1: [fill_k]})
            h_b = jnp.concatenate([acc_a[0:8], xn[40:64]], axis=0).astype(bf16)

            def pre_b(j, r):
                return jnp.concatenate([sav_scr[j], r], axis=0)

            def post_b(j, o):
                return jnp.concatenate([osav[j], o[8:48]], axis=0)

            acc_b = a_pass(lambda j: qkv_cols(h_b, j, 0, 3 * PW), keep_b, fill_b, pre_b, post_b,
                           {0: [fill_v], NP + LAG_O: [fill_t]})
            out = jnp.concatenate([acc_a[8:32], acc_b[0:16], acc_b[24:48]], axis=0)
            x_scr[pl.ds(r0, 64), :] = xs + out
            return acc_b[16:24]

        n_pre = jnp.where(l == 0, NS, 0)
        mem = lax.fori_loop(0, n_pre, functools.partial(step, True), mem_ref[...].astype(f32))
        pl.when(l == 0)(bwo_copy.wait)
        lax.fori_loop(n_pre, NS, functools.partial(step, False), mem)

    def b_layer(l):
        @pl.when(l > 0)
        def _():
            for i in range(NB):
                out_copy(i).wait()

        last = S // 128 - 1
        xl = b1_ln(last)
        b1_pq(last - 1, 1, xnb_scr[1])
        pend = None
        for h in range(2):
            phik = b1_pk(h, xl)
            if pend is not None:
                b1_kvt(*pend)
            lhs = b1_v(h, xl)
            b1_pq(last, h, xl)
            pend = (h, None, phik, lhs)
        b1_kvt(*pend)

        rr = _iota((GR + 8, 2 * GR), 0)
        cc = _iota((GR + 8, 2 * GR), 1)
        m2 = jnp.where(rr < GR, rr // BDH, (rr - GR) // 4) == cc % 2
        for g in range(NG):
            lhs2_scr[g] = jnp.where(m2, kvt_scr[g], 0.0).astype(bf16)

        lo4 = _iota((8, TB), 0) < 4

        def numden(i):
            outs = []
            for g in range(NG):
                phiq = jnp.concatenate([phiq_scr[2 * i, g], phiq_scr[2 * i + 1, g]], axis=1)
                res = jnp.dot(lhs2_scr[g], phiq, preferred_element_type=f32)
                inv = 1.0 / (res[GR:GR + 8] + 1e-6)
                swp = pltpu.roll(inv, 4, 0)
                i0 = jnp.where(lo4, inv, swp)
                i1 = jnp.where(lo4, swp, inv)
                outs += [res[0:8] * i0, res[8:16] * i0, res[16:24] * inv, res[24:32] * i1, res[32:40] * i1]
            return jnp.concatenate(outs, axis=0).T.astype(bf16)

        def proj(i, o):
            rows = pl.ds(i * TB, TB) if isinstance(i, int) else pl.ds(pl.multiple_of(i * TB, TB), TB)
            xnew = x_scr[rows, :] + jnp.dot(o, pltpu.bitcast(bwo_scr[...], bf16), preferred_element_type=f32)
            x_scr[rows, :] = xnew
            xin_scr[rows, :] = xnew.astype(bf16)
            out_copy(i).start()

        o_scr[...] = numden(0)

        def pass2(u, carry):
            o1 = numden(2 * u + 1)
            proj(2 * u, o_scr[...])
            o2 = numden(2 * u + 2)
            proj(2 * u + 1, o1)
            o_scr[...] = o2
            return carry

        lax.fori_loop(0, NB // 2 - 1, pass2, 0)
        o1 = numden(NB - 1)
        proj(NB - 2, o_scr[...])
        proj(NB - 1, o1)

    def layer(l, carry):
        a_layer(l)
        b_layer(l)
        return carry

    lax.fori_loop(0, 2, layer, 0)
    for i in range(NB):
        out_copy(i).wait()


@jax.jit
def pallas_interleave_layers__memory_aug_recurrent_mem_tr__linear_kernel_hedgehog__prompt_kernel(A_x, A_mem0, A_Wq, A_Wk, A_Wv, A_Wo, A_seg_len, B_x, B_wqkv, B_w_phi, B_wo):
    def tr(w):
        return w.transpose(1, 2, 0).reshape(AH * ADH, D)
    out = pl.pallas_call(
        _kernel,
        out_shape=jax.ShapeDtypeStruct((S, D), bf16),
        in_specs=[pl.BlockSpec(memory_space=pl.ANY)] * 10,
        out_specs=pl.BlockSpec(memory_space=pl.ANY),
        scratch_shapes=[
            pltpu.VMEM((S, D), f32),
            pltpu.VMEM((NP, 16, 3 * PW), bf16),
            pltpu.VMEM((NP + 1, D // 2, 3 * PW), u32),
            pltpu.VMEM((NP, PW // 2, D), u32),
            pltpu.VMEM((3, D // 2, D), u32),
            pltpu.VMEM((D // 2, 3 * D), u32),
            pltpu.VMEM((D // 2, D), u32),
            pltpu.VMEM((S // 128, NG, 2 * GR, 128), bf16),
            pltpu.VMEM((NG, GR + 8, 2 * GR), f32),
            pltpu.VMEM((NG, GR + 8, 2 * GR), bf16),
            pltpu.VMEM((S, D), bf16),
            pltpu.VMEM((3, NP + 1, PW // 2, D), u32),
            pltpu.VMEM((NS, 16, D), bf16),
            pltpu.VMEM((NS * 16, D), bf16),
            pltpu.VMEM((NP, NS * 16, PC), bf16),
            pltpu.VMEM((2, 128, D), bf16),
            pltpu.VMEM((TB, D), bf16),
            pltpu.VMEM((D, BDH), f32),
            pltpu.VMEM((M, D), bf16),
            pltpu.VMEM((BDH, BDH, BH), bf16),
            pltpu.VMEM((NG // FP, FR, 256), bf16),
            pltpu.SemaphoreType.DMA((SEM_MISC + 6,)),
        ],
        name="fused_layers",
        compiler_params=pltpu.CompilerParams(vmem_limit_bytes=126 * 1024 * 1024),
    )(A_x.reshape(S, D), A_x.reshape(NS, 64, D), A_mem0.reshape(M, D), tr(A_Wq), tr(A_Wk), tr(A_Wv),
      A_Wo.reshape(AH * ADH, D), B_wqkv, B_w_phi.transpose(1, 2, 0), B_wo)
    return out.reshape(1, S, D)
```

```python
import functools
import jax
import jax.numpy as jnp
from jax import lax
from jax.experimental import pallas as pl
from jax.experimental.pallas import tpu as pltpu

S, D = 2048, 640
AH, ADH, M, SEG = 32, 192, 8, 32
NP = AH // 2
PW = 2 * ADH
BH, BDH = 32, 20
NG = BH // 2
GR = 2 * BDH
TB = 256
NB = S // TB
bf16, f32, u32 = jnp.bfloat16, jnp.float32, jnp.uint32
SCALE = ADH ** -0.5
NEG = -1e9
JUNK = -1e30
NT = (((1,), (1,)), ((), ()))
NS = S // 64
PC = 768
NXP = 4
NX0 = 2
WIN = 4
FP = 2
FR = FP * GR
SEM_WO, SEM_OUT, SEM_XPRE = 3 * WIN, 3 * WIN + 1, 3 * WIN + 2
SEM_MISC = SEM_XPRE + NXP
LAG_S, LAG_P, LAG_O = 1, 3, 4


def _pack(v):
    return pltpu.bitcast(v, u32)


def _unpack(v):
    return pltpu.bitcast(v, bf16)


def _layernorm(x):
    m = jnp.mean(x, axis=-1, keepdims=True)
    xc = x - m
    v = jnp.mean(xc * xc, axis=-1, keepdims=True)
    return xc * lax.rsqrt(v + 1e-5)


def _iota(shape, dim):
    return lax.broadcasted_iota(jnp.int32, shape, dim)


def _make_masks():
    r = _iota((48, 96), 0)
    c = _iota((48, 96), 1)
    c = jnp.where(c >= 48, c - 48, c)
    valid_a = c < 40
    keep_a = ((r < 8) | (r >= c)) & valid_a
    fill_a = jnp.where(valid_a, NEG, JUNK).astype(f32)
    lr = jnp.where(r < 16, r, jnp.where(r < 24, r - 16, r - 8))
    lc = jnp.where(c < 16, c, jnp.where(c < 24, c - 16, c - 8))
    valid_b = c >= 8
    keep_b = ((lr < 8) | (lr >= lc)) & valid_b
    fill_b = jnp.where(valid_b, NEG, JUNK).astype(f32)
    return keep_a, fill_a, keep_b, fill_b


def _blockdiag(k):
    ku = pltpu.bitcast(k, u32)
    lo = _iota(ku.shape, 1) < ADH
    z = jnp.zeros_like(ku)
    return pltpu.bitcast(jnp.concatenate([jnp.where(lo, ku, z), jnp.where(lo, z, ku)], axis=0), bf16)


def _attn_scores(q, k):
    return lax.dot_general(q, _blockdiag(k), NT, preferred_element_type=f32)


def _attn_softmax(s, keep, fill):
    s = jnp.where(keep, s * SCALE, fill)
    h0 = _iota((48, 96), 1) < 48
    m0 = jnp.max(jnp.where(h0, s, -jnp.inf), axis=-1, keepdims=True)
    m1 = jnp.max(jnp.where(h0, -jnp.inf, s), axis=-1, keepdims=True)
    e = jnp.exp(s - jnp.where(h0, m0, m1))
    l0 = jnp.sum(jnp.where(h0, e, 0.0), axis=-1, keepdims=True)
    l1 = jnp.sum(jnp.where(h0, 0.0, e), axis=-1, keepdims=True)
    return (e * jnp.where(h0, 1.0 / l0, 1.0 / l1)).astype(bf16)


def _pair_reduce(op, a):
    a = op(a, pltpu.roll(a, 2, 1))
    return op(a, pltpu.roll(a, 4, 1))


def _features(p):
    t = p.shape[-1]
    ng = p.shape[0] // GR
    p4 = p.reshape(ng, 5, 8, t)
    mx = _pair_reduce(jnp.maximum, jnp.max(p4, axis=1))[:, None]
    mn = _pair_reduce(jnp.minimum, jnp.min(p4, axis=1))[:, None]
    ep = jnp.exp(p4 - mx)
    en = jnp.exp(mn - p4)
    pos = ep * (1.0 / _pair_reduce(jnp.add, jnp.sum(ep, axis=1)))[:, None]
    neg = en * (1.0 / _pair_reduce(jnp.add, jnp.sum(en, axis=1)))[:, None]
    return jnp.concatenate([pos, neg], axis=1).reshape(ng, 2 * GR, t).astype(bf16)


def _kernel(x_hbm, x3_hbm, mem_hbm, wq_hbm, wk_hbm, wv_hbm, wo_hbm, bw_hbm, wphi_hbm, bwo_hbm, o_hbm,
            x_scr, sav_scr, wqkv_scr, wo_scr, wb_scr, bw_scr, bwo_scr, phiq_scr, kvt_scr, lhs2_scr,
            xin_scr, stage_scr, xpre_scr, hpre_scr, pre_scr, xnb_scr, o_scr, wphi_scr, mem_ref, wphi_ref, pm_scr, sems):
    w_hbm = tuple(w.bitcast(u32) for w in (wq_hbm, wk_hbm, wv_hbm, wo_hbm))

    def w_copy(j, m):
        dst = wo_scr.at[j] if m == 3 else stage_scr.at[m, j]
        r0 = j * (PW // 2) if isinstance(j, int) else pl.multiple_of(j * (PW // 2), PW // 2)
        sem = sems.at[SEM_WO] if m == 3 else sems.at[m * WIN + (j & (WIN - 1))]
        return pltpu.make_async_copy(w_hbm[m].at[pl.ds(r0, PW // 2), :], dst, sem)

    def out_copy(i):
        return pltpu.make_async_copy(xin_scr.at[pl.ds(i * TB, TB), :], o_hbm.at[pl.ds(i * TB, TB), :],
                                     sems.at[SEM_OUT])

    def xpre_copy(q):
        steps = pl.ds(q * (NS // NXP), NS // NXP)
        return pltpu.make_async_copy(x3_hbm.at[steps, pl.ds(24, 16), :], xpre_scr.at[steps], sems.at[SEM_XPRE + q])

    x_first = pltpu.make_async_copy(x_hbm.at[pl.ds(0, NX0 * 64), :], xin_scr.at[pl.ds(0, NX0 * 64), :], sems.at[SEM_MISC])
    x_rest = pltpu.make_async_copy(x_hbm.at[pl.ds(NX0 * 64, S - NX0 * 64), :],
                                   xin_scr.at[pl.ds(NX0 * 64, S - NX0 * 64), :], sems.at[SEM_MISC + 1])
    bw_copy = pltpu.make_async_copy(bw_hbm.bitcast(u32), bw_scr, sems.at[SEM_MISC + 2])
    bwo_copy = pltpu.make_async_copy(bwo_hbm.bitcast(u32), bwo_scr, sems.at[SEM_MISC + 3])
    mem_copy = pltpu.make_async_copy(mem_hbm, mem_ref, sems.at[SEM_MISC + 4])
    wphi_copy = pltpu.make_async_copy(wphi_hbm, wphi_ref, sems.at[SEM_MISC + 5])

    def loop(lo, hi, fn):
        lax.fori_loop(lo, hi, lambda i, c: (fn(i), c)[1], 0)

    def start_qkv(j):
        w_copy(j, 0).start()
        w_copy(j, 1).start()
        w_copy(j - 1, 2).start()

    wphi_copy.start()
    for q in range(NXP):
        xpre_copy(q).start()
    w_copy(0, 0).start()
    w_copy(0, 1).start()
    loop(1, WIN, start_qkv)

    x_scr[0:128, :] = jnp.zeros((128, D), f32)
    xnb_scr[...] = jnp.zeros(xnb_scr.shape, bf16)

    def hpre_chunk(q):
        xpre_copy(q).wait()
        xq = xpre_scr[pl.ds(q * (NS // NXP), NS // NXP)].reshape(128, D).astype(f32)
        hpre_scr[pl.ds(pl.multiple_of(q * 128, 128), 128), :] = _layernorm(xq).astype(bf16)

    loop(0, NXP, hpre_chunk)

    def relayout(j, m):
        for t in range(D // 128):
            blk = pltpu.bitcast(stage_scr[m, j, :, t * 128:(t + 1) * 128], bf16)
            wqkv_scr[j, t * 64:(t + 1) * 64, m * PW:(m + 1) * PW] = pltpu.bitcast(blk.T, u32)

    def weight_step(j):
        @pl.when(j < NP)
        def _():
            w_copy(j, 0).wait()
            w_copy(j, 1).wait()

        w_copy(j - 1, 2).wait()
        nxt = j + WIN - 1

        @pl.when(nxt < NP)
        def _():
            w_copy(jnp.minimum(nxt, NP - 1), 0).start()
            w_copy(jnp.minimum(nxt, NP - 1), 1).start()

        pl.when(nxt <= NP)(lambda: w_copy(jnp.minimum(nxt, NP) - 1, 2).start())
        pl.when(nxt == NP)(bw_copy.start)
        w_copy(j - 1, 3).start()
        pre_scr[j - 1] = _pack(jnp.dot(hpre_scr[...], _unpack(wqkv_scr[j - 1, :, 0:PC]),
                                       preferred_element_type=f32).astype(bf16))
        relayout(j, 0)
        relayout(j, 1)
        relayout(j - 1, 2)

    def fold_window(t):
        return 128 * (FR * t // 128), 128 * -(-FR * (t + 1) // 128)

    def fold_matrix(t):
        lo, hi = fold_window(t)
        r = _iota((FR, hi - lo), 0)
        c = _iota((FR, hi - lo), 1) + (lo - FR * t)
        same_head = (c >= 0) & (2 * (r // GR) + r % 2 == jnp.maximum(c, 0) // BDH)
        rf = _iota((FR, BDH), 0) % GR
        et = (_iota((FR, BDH), 1) == 4 * (rf // 8) + (rf % 8) // 2).astype(bf16)
        pm = lax.dot_general(et, wphi_scr[lo:hi, :].astype(bf16), NT, preferred_element_type=f32)
        return jnp.where(same_head, pm, 0.0).astype(bf16)

    wphi_copy.wait()
    for e in range(BDH):
        wphi_scr[pl.ds(e, BH, stride=BDH), :] = wphi_ref[e].astype(f32).T
    for t in range(NG // FP):
        lo, hi = fold_window(t)
        pm_scr[t, :, 0:hi - lo] = fold_matrix(t)

    w_copy(0, 0).wait()
    w_copy(0, 1).wait()
    relayout(0, 0)
    relayout(0, 1)
    loop(1, NP + 1, weight_step)

    x_first.start()
    mem_copy.start()
    bw_copy.wait()
    for t in range(NG // FP):
        lo, hi = fold_window(t)
        for m in range(2):
            w = pltpu.bitcast(bw_scr[:, m * D + lo:m * D + hi], bf16)
            wb_scr[m, t * FR // 2:(t + 1) * FR // 2, :] = pltpu.bitcast(
                lax.dot_general(pm_scr[t, :, 0:hi - lo], w, NT, preferred_element_type=f32).astype(bf16), u32)
    for t in range(D // 128):
        w = pltpu.bitcast(bw_scr[:, 2 * D + 128 * t:2 * D + 128 * (t + 1)], bf16)
        wb_scr[2, t * 64:(t + 1) * 64, :] = pltpu.bitcast(w.T, u32)

    loop(0, NP, lambda j: w_copy(j, 3).wait())
    x_rest.start()
    bwo_copy.start()
    x_first.wait()
    mem_copy.wait()

    HB = NG // 2
    ones = jnp.ones((HB, 8, 128), f32)

    def b1_w(m, h):
        r0 = h * 160 if isinstance(h, int) else pl.multiple_of(h * 160, 160)
        return _unpack(wb_scr[m, pl.ds(r0, 160), :])

    def b1_pk(h, xn):
        pk = jnp.dot(b1_w(1, h), xn, preferred_element_type=f32)
        return _features(pk)

    def b1_v(h, xn):
        vt = jnp.dot(b1_w(2, h), xn, preferred_element_type=f32)
        return jnp.concatenate([vt.reshape(HB, GR, 128), ones], axis=1).astype(bf16)

    def b1_pq(b, h, xn):
        pq = jnp.dot(b1_w(0, h), xn, preferred_element_type=f32)
        phiq_scr[b, pl.ds(pl.multiple_of(h * HB, HB), HB)] = _features(pq)

    def b1_kvt(h, valid, phik, lhs):
        for g in range(HB):
            t = lax.dot_general(lhs[g], phik[g], NT, preferred_element_type=f32)
            if valid is not None:
                t = jnp.where(valid, t, 0.0)
            kvt_scr[h * HB + g] += t

    def b1_ln(b):
        return _layernorm(x_scr[pl.ds(pl.multiple_of(b * 128, 128), 128), :]).astype(bf16).T

    def qkv_cols(h, j, lo, hi):
        w = _unpack(wqkv_scr[j, :, lo:hi])
        return jnp.dot(h, w, preferred_element_type=f32).astype(bf16)

    def a_pass(qkv, keep, fill, pre, post, hooks):
        def oproj(j, o):
            return jnp.dot(o, _unpack(wo_scr[j]), preferred_element_type=f32)

        rs, ws, ss, os_ = {}, {}, {}, {}
        acc = None
        for i in range(NP + LAG_O + 1):
            for fn in hooks.get(i, ()):
                fn()
            if i < NP:
                rs[i] = qkv(i)
            j = i - LAG_S
            if 0 <= j < NP:
                ws[j] = pre(j, rs.pop(j))
                ss[j] = _attn_scores(ws[j][:, 0:PW], ws[j][:, PW:2 * PW])
            j = i - LAG_P
            if 0 <= j < NP:
                p = _attn_softmax(ss.pop(j), keep, fill)
                vbd = _blockdiag(ws.pop(j)[:, 2 * PW:3 * PW])
                o = jnp.dot(p, vbd, preferred_element_type=f32)
                os_[j] = post(j, o).astype(bf16)
            j = i - LAG_O
            if 0 <= j < NP:
                t = oproj(j, os_.pop(j))
                acc = t if acc is None else acc + t
        return acc

    def a_layer(l):
        keep_a, fill_a, keep_b, fill_b = _make_masks()
        kvt_scr[...] = jnp.zeros_like(kvt_scr)

        def step(use_pre, it, mem):
            r0 = pl.multiple_of(it * 64, 64)
            if use_pre:
                pl.when(it == NX0)(x_rest.wait)
                xs = xin_scr[pl.ds(r0, 64), :].astype(f32)
            else:
                xs = x_scr[pl.ds(r0, 64), :]
            xn = _layernorm(xs)
            h_a = jnp.concatenate([mem, xn[0:40]], axis=0).astype(bf16)
            osav = {}

            hq = jnp.maximum(it - 3, 0)
            hk = jnp.maximum(it - 2, 0)
            st = {}

            def fill_q():
                b1_pq(hq >> 1, hq & 1, xnb_scr[...])

            def fill_ln():
                xnb_scr[...] = b1_ln(hk >> 1)

            def fill_k():
                st["phik"] = b1_pk(hk & 1, xnb_scr[...])

            def fill_v():
                st["lhs"] = b1_v(hk & 1, xnb_scr[...])

            def fill_t():
                b1_kvt(hk & 1, it >= 2, st["phik"], st["lhs"])

            def qkv_a(j):
                if use_pre:
                    return qkv_cols(h_a[0:32], j, 0, PC), qkv_cols(h_a, j, PC, 3 * PW)
                return qkv_cols(h_a, j, 0, 3 * PW)

            def pre_a(j, r):
                if use_pre:
                    sv = _unpack(pre_scr[j, pl.ds(pl.multiple_of(it * 8, 8), 8), :])
                    sav_scr[j, :, 0:PC] = _pack(sv)
                    sav_scr[j, :, PC:] = _pack(r[1][32:48])
                    return jnp.concatenate([jnp.concatenate([r[0], sv], axis=0), r[1]], axis=1)
                sav_scr[j] = _pack(r[32:48])
                return r

            def post_a(j, o):
                osav[j] = o[32:40]
                return o[0:32]

            acc_a = a_pass(qkv_a, keep_a, fill_a, pre_a, post_a,
                           {0: [fill_q], 10: [fill_ln], NP + 1: [fill_k]})
            h_b = jnp.concatenate([acc_a[0:8], xn[40:64]], axis=0).astype(bf16)

            def pre_b(j, r):
                return jnp.concatenate([_unpack(sav_scr[j]), r], axis=0)

            def post_b(j, o):
                return jnp.concatenate([osav[j], o[8:48]], axis=0)

            acc_b = a_pass(lambda j: qkv_cols(h_b, j, 0, 3 * PW), keep_b, fill_b, pre_b, post_b,
                           {0: [fill_v], NP + LAG_O: [fill_t]})
            out = jnp.concatenate([acc_a[8:32], acc_b[0:16], acc_b[24:48]], axis=0)
            x_scr[pl.ds(r0, 64), :] = xs + out
            return acc_b[16:24]

        n_pre = jnp.where(l == 0, NS, 0)
        mem = lax.fori_loop(0, n_pre, functools.partial(step, True), mem_ref[...].astype(f32))
        pl.when(l == 0)(bwo_copy.wait)
        lax.fori_loop(n_pre, NS, functools.partial(step, False), mem)

    def b_layer(l):
        @pl.when(l > 0)
        def _():
            for i in range(NB):
                out_copy(i).wait()

        last = S // 128 - 1
        xl = b1_ln(last)
        b1_pq(last - 1, 1, xnb_scr[...])
        pend = None
        for h in range(2):
            phik = b1_pk(h, xl)
            if pend is not None:
                b1_kvt(*pend)
            lhs = b1_v(h, xl)
            b1_pq(last, h, xl)
            pend = (h, None, phik, lhs)
        b1_kvt(*pend)

        rr = _iota((GR + 8, 2 * GR), 0)
        cc = _iota((GR + 8, 2 * GR), 1)
        m2 = jnp.where(rr < GR, rr // BDH, (rr - GR) // 4) == cc % 2
        for g in range(NG):
            lhs2_scr[g] = _pack(jnp.where(m2, kvt_scr[g], 0.0).astype(bf16))

        lo4 = _iota((8, TB), 0) < 4

        def numden(i):
            outs = []
            for g in range(NG):
                phiq = jnp.concatenate([phiq_scr[2 * i, g], phiq_scr[2 * i + 1, g]], axis=1)
                res = jnp.dot(_unpack(lhs2_scr[g]), phiq, preferred_element_type=f32)
                inv = 1.0 / (res[GR:GR + 8] + 1e-6)
                swp = pltpu.roll(inv, 4, 0)
                i0 = jnp.where(lo4, inv, swp)
                i1 = jnp.where(lo4, swp, inv)
                outs += [res[0:8] * i0, res[8:16] * i0, res[16:24] * inv, res[24:32] * i1, res[32:40] * i1]
            return jnp.concatenate(outs, axis=0).T.astype(bf16)

        def proj(i, o):
            rows = pl.ds(i * TB, TB) if isinstance(i, int) else pl.ds(pl.multiple_of(i * TB, TB), TB)
            xnew = x_scr[rows, :] + jnp.dot(o, _unpack(bwo_scr[...]), preferred_element_type=f32)
            x_scr[rows, :] = xnew
            xin_scr[rows, :] = xnew.astype(bf16)
            out_copy(i).start()

        o_scr[...] = _pack(numden(0))

        def pass2(u, carry):
            o1 = numden(2 * u + 1)
            proj(2 * u, _unpack(o_scr[...]))
            o2 = numden(2 * u + 2)
            proj(2 * u + 1, o1)
            o_scr[...] = _pack(o2)
            return carry

        lax.fori_loop(0, NB // 2 - 1, pass2, 0)
        o1 = numden(NB - 1)
        proj(NB - 2, _unpack(o_scr[...]))
        proj(NB - 1, o1)

    def layer(l, carry):
        a_layer(l)
        b_layer(l)
        return carry

    lax.fori_loop(0, 2, layer, 0)
    for i in range(NB):
        out_copy(i).wait()


@jax.jit
def pallas_interleave_layers__memory_aug_recurrent_mem_tr__linear_kernel_hedgehog__prompt_kernel(A_x, A_mem0, A_Wq, A_Wk, A_Wv, A_Wo, A_seg_len, B_x, B_wqkv, B_w_phi, B_wo):
    def tr(w):
        return w.transpose(1, 2, 0).reshape(AH * ADH, D)
    out = pl.pallas_call(
        _kernel,
        out_shape=jax.ShapeDtypeStruct((S, D), bf16),
        in_specs=[pl.BlockSpec(memory_space=pl.ANY)] * 10,
        out_specs=pl.BlockSpec(memory_space=pl.ANY),
        scratch_shapes=[
            pltpu.VMEM((S, D), f32),
            pltpu.VMEM((NP, 8, 3 * PW), u32),
            pltpu.VMEM((NP + 1, D // 2, 3 * PW), u32),
            pltpu.VMEM((NP, PW // 2, D), u32),
            pltpu.VMEM((3, D // 2, D), u32),
            pltpu.VMEM((D // 2, 3 * D), u32),
            pltpu.VMEM((D // 2, D), u32),
            pltpu.VMEM((S // 128, NG, 2 * GR, 128), bf16),
            pltpu.VMEM((NG, GR + 8, 2 * GR), f32),
            pltpu.VMEM((NG, GR // 2 + 4, 2 * GR), u32),
            pltpu.VMEM((S, D), bf16),
            pltpu.VMEM((3, NP + 1, PW // 2, D), u32),
            pltpu.VMEM((NS, 16, D), bf16),
            pltpu.VMEM((NS * 16, D), bf16),
            pltpu.VMEM((NP, NS * 8, PC), u32),
            pltpu.VMEM((D, 128), bf16),
            pltpu.VMEM((TB // 2, D), u32),
            pltpu.VMEM((D, BDH), f32),
            pltpu.VMEM((M, D), bf16),
            pltpu.VMEM((BDH, BDH, BH), bf16),
            pltpu.VMEM((NG // FP, FR, 256), bf16),
            pltpu.SemaphoreType.DMA((SEM_MISC + 6,)),
        ],
        name="fused_layers",
        compiler_params=pltpu.CompilerParams(vmem_limit_bytes=126 * 1024 * 1024),
    )(A_x.reshape(S, D), A_x.reshape(NS, 64, D), A_mem0.reshape(M, D), tr(A_Wq), tr(A_Wk), tr(A_Wv),
      A_Wo.reshape(AH * ADH, D), B_wqkv, B_w_phi.transpose(1, 2, 0), B_wo)
    return out.reshape(1, S, D)
```

```python
import functools
import jax
import jax.numpy as jnp
from jax import lax
from jax.experimental import pallas as pl
from jax.experimental.pallas import tpu as pltpu

S, D = 2048, 640
AH, ADH, M, SEG = 32, 192, 8, 32
NP = AH // 2
PW = 2 * ADH
BH, BDH = 32, 20
NG = BH // 2
GR = 2 * BDH
TB = 256
NB = S // TB
bf16, f32, u32 = jnp.bfloat16, jnp.float32, jnp.uint32
SCALE = ADH ** -0.5
LOG2E = 1.4426950408889634
NEG = -1e9 / SCALE
JUNK = -1e30
NT = (((1,), (1,)), ((), ()))
NS = S // 64
PC = 768
NXP = 4
NX0 = 2
WIN = 4
FP = 2
FR = FP * GR
SEM_WO, SEM_OUT, SEM_XPRE = 3 * WIN, 3 * WIN + 1, 3 * WIN + 2
SEM_MISC = SEM_XPRE + NXP
LAG_S, LAG_P, LAG_O = 1, 3, 4


def _pack(v):
    return pltpu.bitcast(v, u32)


def _unpack(v):
    return pltpu.bitcast(v, bf16)


def _recip(x):
    r = pl.reciprocal(x, approx=True)
    return r * (2.0 - x * r)


def _layernorm(x):
    m = jnp.mean(x, axis=-1, keepdims=True)
    xc = x - m
    v = jnp.mean(xc * xc, axis=-1, keepdims=True)
    return xc * lax.rsqrt(v + 1e-5)


def _iota(shape, dim):
    return lax.broadcasted_iota(jnp.int32, shape, dim)


def _make_masks():
    r = _iota((48, 96), 0)
    c = _iota((48, 96), 1)
    c = jnp.where(c >= 48, c - 48, c)
    valid_a = c < 40
    keep_a = ((r < 8) | (r >= c)) & valid_a
    fill_a = jnp.where(valid_a, NEG, JUNK).astype(f32)
    lr = jnp.where(r < 16, r, jnp.where(r < 24, r - 16, r - 8))
    lc = jnp.where(c < 16, c, jnp.where(c < 24, c - 16, c - 8))
    valid_b = c >= 8
    keep_b = ((lr < 8) | (lr >= lc)) & valid_b
    fill_b = jnp.where(valid_b, NEG, JUNK).astype(f32)
    return keep_a, fill_a, keep_b, fill_b


def _blockdiag(k):
    ku = pltpu.bitcast(k, u32)
    lo = _iota(ku.shape, 1) < ADH
    z = jnp.zeros_like(ku)
    return pltpu.bitcast(jnp.concatenate([jnp.where(lo, ku, z), jnp.where(lo, z, ku)], axis=0), bf16)


def _attn_scores(q, k):
    return lax.dot_general(q, _blockdiag(k), NT, preferred_element_type=f32)


def _attn_softmax(s, keep, fill):
    s = jnp.where(keep, s, fill)
    h0 = _iota((48, 96), 1) < 48
    m0 = jnp.max(jnp.where(h0, s, -jnp.inf), axis=-1, keepdims=True)
    m1 = jnp.max(jnp.where(h0, -jnp.inf, s), axis=-1, keepdims=True)
    e = jnp.exp2((s - jnp.where(h0, m0, m1)) * (SCALE * LOG2E))
    l0 = jnp.sum(jnp.where(h0, e, 0.0), axis=-1, keepdims=True)
    l1 = jnp.sum(jnp.where(h0, 0.0, e), axis=-1, keepdims=True)
    return (e * jnp.where(h0, _recip(l0), _recip(l1))).astype(bf16)


def _pair_reduce(op, a):
    a = op(a, pltpu.roll(a, 2, 1))
    return op(a, pltpu.roll(a, 4, 1))


def _features(p):
    t = p.shape[-1]
    ng = p.shape[0] // GR
    p4 = p.reshape(ng, 5, 8, t)
    mx = _pair_reduce(jnp.maximum, jnp.max(p4, axis=1))[:, None]
    mn = _pair_reduce(jnp.minimum, jnp.min(p4, axis=1))[:, None]
    ep = jnp.exp(p4 - mx)
    en = jnp.exp(mn - p4)
    pos = ep * _recip(_pair_reduce(jnp.add, jnp.sum(ep, axis=1)))[:, None]
    neg = en * _recip(_pair_reduce(jnp.add, jnp.sum(en, axis=1)))[:, None]
    return jnp.concatenate([pos, neg], axis=1).reshape(ng, 2 * GR, t).astype(bf16)


def _kernel(x_hbm, x3_hbm, mem_hbm, wq_hbm, wk_hbm, wv_hbm, wo_hbm, bw_hbm, wphi_hbm, bwo_hbm, o_hbm,
            x_scr, sav_scr, wqkv_scr, wo_scr, wb_scr, bw_scr, bwo_scr, phiq_scr, kvt_scr, lhs2_scr,
            xin_scr, stage_scr, xpre_scr, hpre_scr, pre_scr, xnb_scr, o_scr, wphi_scr, mem_ref, wphi_ref, pm_scr, sems):
    w_hbm = tuple(w.bitcast(u32) for w in (wq_hbm, wk_hbm, wv_hbm, wo_hbm))

    def w_copy(j, m):
        dst = wo_scr.at[j] if m == 3 else stage_scr.at[m, j]
        r0 = j * (PW // 2) if isinstance(j, int) else pl.multiple_of(j * (PW // 2), PW // 2)
        sem = sems.at[SEM_WO] if m == 3 else sems.at[m * WIN + (j & (WIN - 1))]
        return pltpu.make_async_copy(w_hbm[m].at[pl.ds(r0, PW // 2), :], dst, sem)

    def out_copy(i):
        return pltpu.make_async_copy(xin_scr.at[pl.ds(i * TB, TB), :], o_hbm.at[pl.ds(i * TB, TB), :],
                                     sems.at[SEM_OUT])

    def xpre_copy(q):
        steps = pl.ds(q * (NS // NXP), NS // NXP)
        return pltpu.make_async_copy(x3_hbm.at[steps, pl.ds(24, 16), :], xpre_scr.at[steps], sems.at[SEM_XPRE + q])

    x_first = pltpu.make_async_copy(x_hbm.at[pl.ds(0, NX0 * 64), :], xin_scr.at[pl.ds(0, NX0 * 64), :], sems.at[SEM_MISC])
    x_rest = pltpu.make_async_copy(x_hbm.at[pl.ds(NX0 * 64, S - NX0 * 64), :],
                                   xin_scr.at[pl.ds(NX0 * 64, S - NX0 * 64), :], sems.at[SEM_MISC + 1])
    bw_copy = pltpu.make_async_copy(bw_hbm.bitcast(u32), bw_scr, sems.at[SEM_MISC + 2])
    bwo_copy = pltpu.make_async_copy(bwo_hbm.bitcast(u32), bwo_scr, sems.at[SEM_MISC + 3])
    mem_copy = pltpu.make_async_copy(mem_hbm, mem_ref, sems.at[SEM_MISC + 4])
    wphi_copy = pltpu.make_async_copy(wphi_hbm, wphi_ref, sems.at[SEM_MISC + 5])

    def loop(lo, hi, fn):
        lax.fori_loop(lo, hi, lambda i, c: (fn(i), c)[1], 0)

    def start_qkv(j):
        w_copy(j, 0).start()
        w_copy(j, 1).start()
        w_copy(j - 1, 2).start()

    wphi_copy.start()
    for q in range(NXP):
        xpre_copy(q).start()
    w_copy(0, 0).start()
    w_copy(0, 1).start()
    loop(1, WIN, start_qkv)

    x_scr[0:128, :] = jnp.zeros((128, D), f32)
    xnb_scr[...] = jnp.zeros(xnb_scr.shape, bf16)

    def hpre_chunk(q):
        xpre_copy(q).wait()
        xq = xpre_scr[pl.ds(q * (NS // NXP), NS // NXP)].reshape(128, D).astype(f32)
        hpre_scr[pl.ds(pl.multiple_of(q * 128, 128), 128), :] = _layernorm(xq).astype(bf16)

    loop(0, NXP, hpre_chunk)

    def relayout(j, m):
        for t in range(D // 128):
            blk = pltpu.bitcast(stage_scr[m, j, :, t * 128:(t + 1) * 128], bf16)
            wqkv_scr[j, t * 64:(t + 1) * 64, m * PW:(m + 1) * PW] = pltpu.bitcast(blk.T, u32)

    def weight_step(j):
        @pl.when(j < NP)
        def _():
            w_copy(j, 0).wait()
            w_copy(j, 1).wait()

        w_copy(j - 1, 2).wait()
        nxt = j + WIN - 1

        @pl.when(nxt < NP)
        def _():
            w_copy(jnp.minimum(nxt, NP - 1), 0).start()
            w_copy(jnp.minimum(nxt, NP - 1), 1).start()

        pl.when(nxt <= NP)(lambda: w_copy(jnp.minimum(nxt, NP) - 1, 2).start())
        pl.when(nxt == NP)(bw_copy.start)
        w_copy(j - 1, 3).start()
        pre_scr[j - 1] = _pack(jnp.dot(hpre_scr[...], _unpack(wqkv_scr[j - 1, :, 0:PC]),
                                       preferred_element_type=f32).astype(bf16))
        relayout(j, 0)
        relayout(j, 1)
        relayout(j - 1, 2)

    def fold_window(t):
        return 128 * (FR * t // 128), 128 * -(-FR * (t + 1) // 128)

    def fold_matrix(t):
        lo, hi = fold_window(t)
        r = _iota((FR, hi - lo), 0)
        c = _iota((FR, hi - lo), 1) + (lo - FR * t)
        same_head = (c >= 0) & (2 * (r // GR) + r % 2 == jnp.maximum(c, 0) // BDH)
        rf = _iota((FR, BDH), 0) % GR
        et = (_iota((FR, BDH), 1) == 4 * (rf // 8) + (rf % 8) // 2).astype(bf16)
        pm = lax.dot_general(et, wphi_scr[lo:hi, :].astype(bf16), NT, preferred_element_type=f32)
        return jnp.where(same_head, pm, 0.0).astype(bf16)

    wphi_copy.wait()
    for e in range(BDH):
        wphi_scr[pl.ds(e, BH, stride=BDH), :] = wphi_ref[e].astype(f32).T
    for t in range(NG // FP):
        lo, hi = fold_window(t)
        pm_scr[t, :, 0:hi - lo] = fold_matrix(t)

    w_copy(0, 0).wait()
    w_copy(0, 1).wait()
    relayout(0, 0)
    relayout(0, 1)
    loop(1, NP + 1, weight_step)

    x_first.start()
    mem_copy.start()
    bw_copy.wait()
    for t in range(NG // FP):
        lo, hi = fold_window(t)
        for m in range(2):
            w = pltpu.bitcast(bw_scr[:, m * D + lo:m * D + hi], bf16)
            wb_scr[m, t * FR // 2:(t + 1) * FR // 2, :] = pltpu.bitcast(
                lax.dot_general(pm_scr[t, :, 0:hi - lo], w, NT, preferred_element_type=f32).astype(bf16), u32)
    for t in range(D // 128):
        w = pltpu.bitcast(bw_scr[:, 2 * D + 128 * t:2 * D + 128 * (t + 1)], bf16)
        wb_scr[2, t * 64:(t + 1) * 64, :] = pltpu.bitcast(w.T, u32)

    loop(0, NP, lambda j: w_copy(j, 3).wait())
    x_rest.start()
    bwo_copy.start()
    x_first.wait()
    mem_copy.wait()

    HB = NG // 2
    ones = jnp.ones((HB, 8, 128), f32)

    def b1_w(m, h):
        r0 = h * 160 if isinstance(h, int) else pl.multiple_of(h * 160, 160)
        return _unpack(wb_scr[m, pl.ds(r0, 160), :])

    def b1_pk(h, xn):
        pk = jnp.dot(b1_w(1, h), xn, preferred_element_type=f32)
        return _features(pk)

    def b1_v(h, xn):
        vt = jnp.dot(b1_w(2, h), xn, preferred_element_type=f32)
        return jnp.concatenate([vt.reshape(HB, GR, 128), ones], axis=1).astype(bf16)

    def b1_pq(b, h, xn):
        pq = jnp.dot(b1_w(0, h), xn, preferred_element_type=f32)
        phiq_scr[b, pl.ds(pl.multiple_of(h * HB, HB), HB)] = _features(pq)

    def b1_kvt(h, valid, phik, lhs):
        for g in range(HB):
            t = lax.dot_general(lhs[g], phik[g], NT, preferred_element_type=f32)
            if valid is not None:
                t = jnp.where(valid, t, 0.0)
            kvt_scr[h * HB + g] += t

    def b1_ln(b):
        return _layernorm(x_scr[pl.ds(pl.multiple_of(b * 128, 128), 128), :]).astype(bf16).T

    def qkv_cols(h, j, lo, hi):
        w = _unpack(wqkv_scr[j, :, lo:hi])
        return jnp.dot(h, w, preferred_element_type=f32).astype(bf16)

    def a_pass(qkv, keep, fill, pre, post, hooks):
        def oproj(j, o):
            return jnp.dot(o, _unpack(wo_scr[j]), preferred_element_type=f32)

        rs, ws, ss, os_ = {}, {}, {}, {}
        acc = None
        for i in range(NP + LAG_O + 1):
            for fn in hooks.get(i, ()):
                fn()
            if i < NP:
                rs[i] = qkv(i)
            j = i - LAG_S
            if 0 <= j < NP:
                ws[j] = pre(j, rs.pop(j))
                ss[j] = _attn_scores(ws[j][:, 0:PW], ws[j][:, PW:2 * PW])
            j = i - LAG_P
            if 0 <= j < NP:
                p = _attn_softmax(ss.pop(j), keep, fill)
                vbd = _blockdiag(ws.pop(j)[:, 2 * PW:3 * PW])
                o = jnp.dot(p, vbd, preferred_element_type=f32)
                os_[j] = post(j, o).astype(bf16)
            j = i - LAG_O
            if 0 <= j < NP:
                t = oproj(j, os_.pop(j))
                acc = t if acc is None else acc + t
        return acc

    def a_layer(l):
        keep_a, fill_a, keep_b, fill_b = _make_masks()
        kvt_scr[...] = jnp.zeros_like(kvt_scr)

        def step(use_pre, it, mem):
            r0 = pl.multiple_of(it * 64, 64)
            if use_pre:
                pl.when(it == NX0)(x_rest.wait)
                xs = xin_scr[pl.ds(r0, 64), :].astype(f32)
            else:
                xs = x_scr[pl.ds(r0, 64), :]
            xn = _layernorm(xs)
            h_a = jnp.concatenate([mem, xn[0:40]], axis=0).astype(bf16)
            osav = {}

            hq = jnp.maximum(it - 3, 0)
            hk = jnp.maximum(it - 2, 0)
            st = {}

            def fill_q():
                b1_pq(hq >> 1, hq & 1, xnb_scr[...])

            def fill_ln():
                xnb_scr[...] = b1_ln(hk >> 1)

            def fill_k():
                st["phik"] = b1_pk(hk & 1, xnb_scr[...])

            def fill_v():
                st["lhs"] = b1_v(hk & 1, xnb_scr[...])

            def fill_t():
                b1_kvt(hk & 1, it >= 2, st["phik"], st["lhs"])

            def qkv_a(j):
                if use_pre:
                    return qkv_cols(h_a[0:32], j, 0, PC), qkv_cols(h_a, j, PC, 3 * PW)
                return qkv_cols(h_a, j, 0, 3 * PW)

            def pre_a(j, r):
                if use_pre:
                    sv = _unpack(pre_scr[j, pl.ds(pl.multiple_of(it * 8, 8), 8), :])
                    sav_scr[j, :, 0:PC] = _pack(sv)
                    sav_scr[j, :, PC:] = _pack(r[1][32:48])
                    return jnp.concatenate([jnp.concatenate([r[0], sv], axis=0), r[1]], axis=1)
                sav_scr[j] = _pack(r[32:48])
                return r

            def post_a(j, o):
                osav[j] = o[32:40]
                return o[0:32]

            acc_a = a_pass(qkv_a, keep_a, fill_a, pre_a, post_a,
                           {0: [fill_q], 10: [fill_ln], NP + 1: [fill_k]})
            h_b = jnp.concatenate([acc_a[0:8], xn[40:64]], axis=0).astype(bf16)

            def pre_b(j, r):
                return jnp.concatenate([_unpack(sav_scr[j]), r], axis=0)

            def post_b(j, o):
                return jnp.concatenate([osav[j], o[8:48]], axis=0)

            acc_b = a_pass(lambda j: qkv_cols(h_b, j, 0, 3 * PW), keep_b, fill_b, pre_b, post_b,
                           {0: [fill_v], NP + LAG_O: [fill_t]})
            out = jnp.concatenate([acc_a[8:32], acc_b[0:16], acc_b[24:48]], axis=0)
            x_scr[pl.ds(r0, 64), :] = xs + out
            return acc_b[16:24]

        n_pre = jnp.where(l == 0, NS, 0)
        mem = lax.fori_loop(0, n_pre, functools.partial(step, True), mem_ref[...].astype(f32))
        pl.when(l == 0)(bwo_copy.wait)
        lax.fori_loop(n_pre, NS, functools.partial(step, False), mem)

    def b_layer(l):
        @pl.when(l > 0)
        def _():
            for i in range(NB):
                out_copy(i).wait()

        last = S // 128 - 1
        xl = b1_ln(last)
        b1_pq(last - 1, 1, xnb_scr[...])
        pend = None
        for h in range(2):
            phik = b1_pk(h, xl)
            if pend is not None:
                b1_kvt(*pend)
            lhs = b1_v(h, xl)
            b1_pq(last, h, xl)
            pend = (h, None, phik, lhs)
        b1_kvt(*pend)

        rr = _iota((GR + 8, 2 * GR), 0)
        cc = _iota((GR + 8, 2 * GR), 1)
        m2 = jnp.where(rr < GR, rr // BDH, (rr - GR) // 4) == cc % 2
        for g in range(NG):
            lhs2_scr[g] = _pack(jnp.where(m2, kvt_scr[g], 0.0).astype(bf16))

        lo4 = _iota((8, TB), 0) < 4

        def numden(i):
            outs = []
            for g in range(NG):
                phiq = jnp.concatenate([phiq_scr[2 * i, g], phiq_scr[2 * i + 1, g]], axis=1)
                res = jnp.dot(_unpack(lhs2_scr[g]), phiq, preferred_element_type=f32)
                inv = _recip(res[GR:GR + 8] + 1e-6)
                swp = pltpu.roll(inv, 4, 0)
                i0 = jnp.where(lo4, inv, swp)
                i1 = jnp.where(lo4, swp, inv)
                outs += [res[0:8] * i0, res[8:16] * i0, res[16:24] * inv, res[24:32] * i1, res[32:40] * i1]
            return jnp.concatenate(outs, axis=0).T.astype(bf16)

        def proj(i, o):
            rows = pl.ds(i * TB, TB) if isinstance(i, int) else pl.ds(pl.multiple_of(i * TB, TB), TB)
            xnew = x_scr[rows, :] + jnp.dot(o, _unpack(bwo_scr[...]), preferred_element_type=f32)
            x_scr[rows, :] = xnew
            xin_scr[rows, :] = xnew.astype(bf16)
            out_copy(i).start()

        o0 = numden(0)
        o1 = numden(1)
        proj(0, o0)
        o_scr[...] = _pack(o1)

        def pass2(u, carry):
            i = 3 * u + 1
            oa = numden(i + 1)
            proj(i, _unpack(o_scr[...]))
            ob = numden(i + 2)
            proj(i + 1, oa)
            oc = numden(i + 3)
            proj(i + 2, ob)
            o_scr[...] = _pack(oc)
            return carry

        lax.fori_loop(0, (NB - 2) // 3, pass2, 0)
        proj(NB - 1, _unpack(o_scr[...]))

    def layer(l, carry):
        a_layer(l)
        b_layer(l)
        return carry

    lax.fori_loop(0, 2, layer, 0)
    for i in range(NB):
        out_copy(i).wait()


@jax.jit
def pallas_interleave_layers__memory_aug_recurrent_mem_tr__linear_kernel_hedgehog__prompt_kernel(A_x, A_mem0, A_Wq, A_Wk, A_Wv, A_Wo, A_seg_len, B_x, B_wqkv, B_w_phi, B_wo):
    def tr(w):
        return w.transpose(1, 2, 0).reshape(AH * ADH, D)
    out = pl.pallas_call(
        _kernel,
        out_shape=jax.ShapeDtypeStruct((S, D), bf16),
        in_specs=[pl.BlockSpec(memory_space=pl.ANY)] * 10,
        out_specs=pl.BlockSpec(memory_space=pl.ANY),
        scratch_shapes=[
            pltpu.VMEM((S, D), f32),
            pltpu.VMEM((NP, 8, 3 * PW), u32),
            pltpu.VMEM((NP + 1, D // 2, 3 * PW), u32),
            pltpu.VMEM((NP, PW // 2, D), u32),
            pltpu.VMEM((3, D // 2, D), u32),
            pltpu.VMEM((D // 2, 3 * D), u32),
            pltpu.VMEM((D // 2, D), u32),
            pltpu.VMEM((S // 128, NG, 2 * GR, 128), bf16),
            pltpu.VMEM((NG, GR + 8, 2 * GR), f32),
            pltpu.VMEM((NG, GR // 2 + 4, 2 * GR), u32),
            pltpu.VMEM((S, D), bf16),
            pltpu.VMEM((3, NP + 1, PW // 2, D), u32),
            pltpu.VMEM((NS, 16, D), bf16),
            pltpu.VMEM((NS * 16, D), bf16),
            pltpu.VMEM((NP, NS * 8, PC), u32),
            pltpu.VMEM((D, 128), bf16),
            pltpu.VMEM((TB // 2, D), u32),
            pltpu.VMEM((D, BDH), f32),
            pltpu.VMEM((M, D), bf16),
            pltpu.VMEM((BDH, BDH, BH), bf16),
            pltpu.VMEM((NG // FP, FR, 256), bf16),
            pltpu.SemaphoreType.DMA((SEM_MISC + 6,)),
        ],
        name="fused_layers",
        compiler_params=pltpu.CompilerParams(vmem_limit_bytes=126 * 1024 * 1024),
    )(A_x.reshape(S, D), A_x.reshape(NS, 64, D), A_mem0.reshape(M, D), tr(A_Wq), tr(A_Wk), tr(A_Wv),
      A_Wo.reshape(AH * ADH, D), B_wqkv, B_w_phi.transpose(1, 2, 0), B_wo)
    return out.reshape(1, S, D)
```
